```python
import os as _os
_os.environ.setdefault("JAX_PLATFORMS", "cpu")
import jax
import jax.numpy as jnp

def _softmax(x, axis=-1):
    return jax.nn.softmax(x, axis=axis)
def _gelu(x):
    return jax.nn.gelu(x, approximate=True)
def _silu(x):
    return jax.nn.silu(x)
def _sigmoid(x):
    return jax.nn.sigmoid(x)
def _layernorm(x, axis=-1, eps=1e-5):
    m = jnp.mean(x, axis=axis, keepdims=True)
    v = jnp.var(x, axis=axis, keepdims=True)
    return (x - m) / jnp.sqrt(v + eps)
def _scatter_add(tgt, idx, src, axis=0):
    return tgt.at[idx].add(src)
def _segment_sum(src, seg, n):
    return jax.ops.segment_sum(src, seg, n)
class _Rng:
    def __init__(self, key):
        self._k = key
    def _next(self):
        self._k, sub = jax.random.split(self._k)
        return sub
    def normal(self, shape):
        return jax.random.normal(self._next(), shape, dtype=jnp.bfloat16)
    def randint(self, lo, hi, shape):
        return jax.random.randint(self._next(), shape, lo, hi, dtype=jnp.int32)
    def uniform(self, shape, lo=0.0, hi=1.0):
        return jax.random.uniform(self._next(), shape, jnp.bfloat16, lo, hi)
    def permutation(self, n):
        return jax.random.permutation(self._next(), n)


kernel_name = 'gated_mix__mha_block__mixer_s_mlp__prompt'

def setup_inputs():
    _rng = _Rng(jax.random.key(int.from_bytes(__import__("os").urandom(4), "little")))
    _w = (lambda a: (lambda t: t.astype(jnp.bfloat16) if jnp.issubdtype(t.dtype, jnp.floating) else t)(jnp.asarray(a)))
    def _A_setup():
        B, S, D, H = 1, 2048, 448, 16
        return {
            "x": _w((lambda *s: _rng.normal(s) * 0.05)(B, S, D)),
            "wqkv": _w((lambda *s: _rng.normal(s) * 0.8)(D, 3 * D)),
            "wo": _w((lambda *s: _rng.normal(s) * 0.05)(D, D)),
        }
    _A_in = _A_setup()

    def _B_setup():
        B, S, D, F = 1, 2048, 448, 1792
        return {
            "x":  _w((lambda *s: _rng.normal(s) * 0.05)(B, S, D)),
            "w1": _w((lambda *s: _rng.normal(s) * 0.2)(D, D) * (D ** -0.5)),
            "w2": _w((lambda *s: _rng.normal(s) * 0.2)(D, D) * (D ** -0.5)),
            "w3": _w((lambda *s: _rng.normal(s) * 0.2)(D, F) * (D ** -0.5)),
            "w4": _w((lambda *s: _rng.normal(s) * 0.2)(F, D) * (F ** -0.5)),
        }
    _B_in = _B_setup()

    return {
        "A_x": _A_in["x"],
        "A_wqkv": _A_in["wqkv"],
        "A_wo": _A_in["wo"],
        "B_x": _B_in["x"],
        "B_w1": _B_in["w1"],
        "B_w2": _B_in["w2"],
        "B_w3": _B_in["w3"],
        "B_w4": _B_in["w4"],
        "gate_w": _w((lambda *s: _rng.normal(s) * 0.05)(448) * 16.0),
    }

def reference(A_x, A_wqkv, A_wo, B_x, B_w1, B_w2, B_w3, B_w4, gate_w):
    def _A_ref(x, wqkv, wo):
        B, S, D = x.shape
        H = 16
        Dh = D // H
        qkv = (lambda x, *d: x.transpose(*d))((x @ wqkv).reshape(B, S, 3, H, Dh), 2, 0, 3, 1, 4)
        q, k, v = qkv[0], qkv[1], qkv[2]
        scores = jnp.einsum("bhqd,bhkd->bhqk", q, k) * (Dh ** -0.5)
        p = _softmax(scores, axis=-1)
        o = jnp.einsum("bhqk,bhkd->bhqd", p, v)
        return (lambda x, *d: x.transpose(*d))(o, 0, 2, 1, 3).reshape(B, S, D) @ wo

    def _B_ref(x, w1, w2, w3, w4):
        B, S, D = x.shape
        h = _gelu(_layernorm(x, axis=-1) @ w1)
        c = D // 4
        g0 = jnp.pad(h[:, :, 0*c:1*c], ((0, 0), (1, 0), (0, 0)))[:, :S, :]
        g1 = jnp.pad(h[:, :, 1*c:2*c], ((0, 0), (0, 1), (0, 0)))[:, 1:, :]
        g2 = jnp.pad(h[:, :, 2*c:3*c], ((0, 0), (2, 0), (0, 0)))[:, :S, :]
        g3 = jnp.pad(h[:, :, 3*c:   ], ((0, 0), (0, 2), (0, 0)))[:, 2:, :]
        hs = jnp.concatenate([g0, g1, g2, g3], axis=-1) @ w2
        x1 = x + hs
        h2 = _gelu(_layernorm(x1, axis=-1) @ w3) @ w4
        return x1 + h2

    x = A_x
    g = _sigmoid((x * gate_w).sum(-1, keepdims=True))
    a = _A_ref(x, A_wqkv, A_wo)
    b = _B_ref(x, B_w1, B_w2, B_w3, B_w4)
    return g * a + (1 - g) * b
```

```python
import functools
import math
import os

import jax
import jax.numpy as jnp
from jax import lax
import jax.experimental.pallas as pl
import jax.experimental.pallas.tpu as pltpu

S, D, H, DH, F = 2048, 448, 16, 28, 1792
NG = 4
GW = 4 * DH
HP = 32
TT = 512
TQ = 512
CK = 128
LAG = int(os.environ.get("LAG", 2))
FC = int(os.environ.get("FC", 256))
U = int(os.environ.get("U", 9))
NB = 3
REP = int(os.environ.get("REP", 1))
REPP = int(os.environ.get("REPP", 1))
REPF = int(os.environ.get("REPF", 1))
C4 = D // 4
NT = S // TT
NQ = S // TQ
NSTEP = NQ * H
NC = S // CK

bf16 = jnp.bfloat16
f32 = jnp.float32
TN = (((0,), (0,)), ((), ()))


def _gelu(x):
    c0 = math.sqrt(2.0 / math.pi)
    inner = x * (c0 + (c0 * 0.044715) * (x * x))
    hx = 0.5 * x
    return hx + hx * jnp.tanh(inner)


def _ln_t(x):
    m = jnp.sum(x, axis=0, keepdims=True) * (1.0 / D)
    xc = x - m
    v = jnp.sum(xc * xc, axis=0, keepdims=True) * (1.0 / D)
    return xc * lax.rsqrt(v + 1e-5)


def _dot(a, b):
    return jnp.dot(a, b, preferred_element_type=f32)


def _dot_tn(a, b):
    return lax.dot_general(a, b, TN, preferred_element_type=f32)


def _kernel(xt_hbm, wqkv_hbm, wo_hbm, w1_hbm, w2_hbm, w3_hbm, w4t_hbm, gw_ref, out_hbm,
            xt_v, wqkv_v, wo_v, w1_v, w2_v, w3_v, w4t_v, out_v, in_sems, x_sems, out_sems,
            wop_s, pad_s, gw_s,
            qt_s, k_s, vt_s, z_s, h_s, ln_s, b_s, s0_s, s1_s, s2_s, ot_s):
    srcs = (w1_hbm, wqkv_hbm, w2_hbm, w3_hbm, w4t_hbm, wo_hbm)
    dsts = (w1_v, wqkv_v, w2_v, w3_v, w4t_v, wo_v)
    cp_w1, cp_wqkv, cp_w2, cp_w3, cp_w4, cp_wo = [
        pltpu.make_async_copy(s_, d_, in_sems.at[i]) for i, (s_, d_) in enumerate(zip(srcs, dsts))]
    cp_x = [pltpu.make_async_copy(xt_hbm.at[:, i * TT:(i + 1) * TT], xt_v.at[:, i * TT:(i + 1) * TT],
                                  x_sems.at[i]) for i in range(NT)]
    cp_x[0].start()
    cp_w1.start()
    for i in range(1, NT):
        cp_x[i].start()
    cp_wqkv.start()
    cp_w2.start()
    cp_wo.start()
    cp_w3.start()
    cp_w4.start()

    qscale = (DH ** -0.5) * math.log2(math.e)

    def mix1(i):
        cols = slice(i * TT, (i + 1) * TT)
        xf = xt_v[:, cols].astype(f32)
        gwc = gw_s[...]
        z_s[:, cols] = jnp.sum(xf * jnp.concatenate([gwc] * (TT // 128), axis=1), axis=0, keepdims=True)
        ln = _ln_t(xf).astype(bf16)
        h = _gelu(_dot_tn(w1_v[...], ln))
        h_s[:, i * TT + 128:(i + 1) * TT + 128] = h.astype(bf16)

    h_s[:, 0:128] = jnp.zeros((D, 128), bf16)
    h_s[:, S + 128:S + 256] = jnp.zeros((D, 128), bf16)
    gw_s[...] = jnp.broadcast_to(gw_ref[...].astype(f32), (128, D)).T
    for sb in (s0_s, s1_s, s2_s):
        sb[0:8, :] = jnp.zeros((8, TQ), f32)
    cp_x[0].wait()
    cp_w1.wait()
    mix1(0)
    cp_x[1].wait()
    cp_x[2].wait()
    mix1(1)
    mix1(2)
    cp_x[3].wait()
    mix1(3)
    cp_wqkv.wait()
    cp_w2.wait()

    def proj(i, carry):
        t0 = pl.multiple_of(i * TT, TT)
        cols = pl.ds(t0, TT)
        xt = xt_v[:, cols]
        hw = h_s[:, pl.ds(t0, TT + 256)]
        hs = jnp.concatenate([
            hw[0 * C4:1 * C4, 127:127 + TT],
            hw[1 * C4:2 * C4, 129:129 + TT],
            hw[2 * C4:3 * C4, 126:126 + TT],
            hw[3 * C4:4 * C4, 130:130 + TT]], axis=0)
        qk = _dot_tn(wqkv_v[:, 0:2 * D], xt)
        qt_s[:, cols] = (qk[0:D, :] * qscale).astype(bf16)
        kt = qk[D:2 * D, :].astype(bf16)
        for g in range(NG):
            k_s[g, cols, :] = kt[GW * g:GW * (g + 1), :].T
        x1 = xt.astype(f32) + _dot_tn(w2_v[...], hs)
        b_s[:, cols] = x1
        ln_s[:, cols] = _ln_t(x1).astype(bf16)
        vt = _dot_tn(wqkv_v[:, 2 * D:3 * D], xt)
        rid = lax.broadcasted_iota(jnp.int32, (HP - DH, TT), 0)
        tail = jnp.where(rid == 0, 1.0, 0.0).astype(f32)
        for h in range(H):
            vt_s[HP * h:HP * (h + 1), cols] = jnp.concatenate(
                [vt[DH * h:DH * (h + 1), :], tail], axis=0).astype(bf16)
        return carry

    lax.fori_loop(0, NT * REPP, lambda i, c: proj(i % NT, c), 0)

    sbuf = (s0_s, s1_s, s2_s)

    def mo(v, n):
        return v if isinstance(v, int) else pl.multiple_of(v, n)

    def step(t1, s1_ref, t2, s2_ref, m2):
        if t1 is not None:
            h1 = t1 % H
            g = h1 // 4
            j = h1 % 4
            q = qt_s[pl.ds(mo(g * GW, 16), GW), pl.ds(mo((t1 // H) * TQ, TQ), TQ)]
            row = lax.broadcasted_iota(jnp.int32, (GW, TQ), 0)
            lo = j * DH
            qm = jnp.where(jnp.logical_and(row >= lo, row < lo + DH), q, jnp.zeros_like(q))
        if t2 is not None:
            h0 = mo((t2 % H) * HP, HP)
        m = None
        acc = None
        for cc in range(NC + LAG):
            if t1 is not None and cc < NC:
                ks = slice(cc * CK, (cc + 1) * CK)
                s = _dot(k_s[g, ks, :], qm)
                s1_ref[ks, :] = s
                mc = jnp.max(s.reshape(CK // 8, 8, TQ), axis=0)
                m = mc if m is None else jnp.maximum(m, mc)
            if t2 is not None and cc >= LAG:
                ks = slice((cc - LAG) * CK, (cc - LAG + 1) * CK)
                p = jnp.exp2(s2_ref[ks, :] - m2).astype(bf16)
                pv = _dot(vt_s[pl.ds(h0, HP), ks], p)
                acc = pv if acc is None else acc + pv
        if t2 is not None:
            inv = 1.0 / acc[DH:DH + 1, :]
            ot_s[pl.ds(h0, HP), pl.ds(mo((t2 // H) * TQ, TQ), TQ)] = (acc * inv).astype(bf16)
        if t1 is not None:
            return jnp.max(m, axis=0, keepdims=True)

    def body(i, m):
        for u in range(U):
            t = i * U + u
            m = step(t + 1, sbuf[(u + 1) % NB], t, sbuf[u % NB], m)
        return m

    niter = (NSTEP - 1) // U
    m = step(0, sbuf[0], None, None, None)
    m = lax.fori_loop(0, niter * REP, lambda i, m: body(i % niter, m), m)
    cp_wo.wait()
    cp_w3.wait()
    cp_w4.wait()
    wo_f = wo_v[...].astype(f32)
    for h in range(H):
        pad_s[HP * h:HP * h + DH, :] = wo_f[DH * h:DH * (h + 1), :]
        pad_s[HP * h + DH:HP * (h + 1), :] = jnp.zeros((HP - DH, D), f32)
    wop_s[...] = pad_s[...].astype(bf16)
    step(None, None, NSTEP - 1, sbuf[(NSTEP - 1) % NB], m)

    def out_copy(i):
        cols = pl.ds(mo(i * TT, TT), TT)
        return pltpu.make_async_copy(out_v.at[:, cols], out_hbm.at[:, cols], out_sems.at[i])

    def ffn(i, carry):
        t0 = pl.multiple_of(i * TT, TT)
        cols = pl.ds(t0, TT)
        ln = ln_s[:, cols]
        a = _dot_tn(wop_s[...], ot_s[:, cols])
        gate = 1.0 / (1.0 + jnp.exp(-z_s[:, cols]))
        acc = b_s[:, cols]
        for fc in range(F // FC):
            gg = _gelu(_dot_tn(w3_v[:, fc * FC:(fc + 1) * FC], ln)).astype(bf16)
            acc = acc + _dot(w4t_v[:, fc * FC:(fc + 1) * FC], gg)
        out_v[:, cols] = (acc + gate * (a - acc)).astype(bf16)
        if REPF == 1:
            out_copy(i).start()
        return carry

    lax.fori_loop(0, NT * REPF, lambda i, c: ffn(i % NT, c), 0)
    for i in range(NT):
        if REPF != 1:
            out_copy(i).start()
        out_copy(i).wait()


@jax.jit
def pallas_gated_mix__mha_block__mixer_s_mlp__prompt_kernel(A_x, A_wqkv, A_wo, B_x, B_w1, B_w2, B_w3, B_w4, gate_w):
    xt = A_x.reshape(S, D).T
    w4t = B_w4.T
    gw = gate_w.reshape(1, D)
    any_spec = pl.BlockSpec(memory_space=pl.ANY)
    out_t = pl.pallas_call(
        _kernel,
        out_shape=jax.ShapeDtypeStruct((D, S), A_x.dtype),
        in_specs=[any_spec] * 7 + [pl.BlockSpec(memory_space=pltpu.VMEM)],
        out_specs=any_spec,
        scratch_shapes=[
            pltpu.VMEM((D, S), bf16),
            pltpu.VMEM((D, 3 * D), bf16),
            pltpu.VMEM((D, D), bf16),
            pltpu.VMEM((D, D), bf16),
            pltpu.VMEM((D, D), bf16),
            pltpu.VMEM((D, F), bf16),
            pltpu.VMEM((D, F), bf16),
            pltpu.VMEM((D, S), bf16),
            pltpu.SemaphoreType.DMA((6,)),
            pltpu.SemaphoreType.DMA((NT,)),
            pltpu.SemaphoreType.DMA((NT,)),
            pltpu.VMEM((H * HP, D), bf16),
            pltpu.VMEM((H * HP, D), f32),
            pltpu.VMEM((D, 128), f32),
            pltpu.VMEM((D, S), bf16),
            pltpu.VMEM((NG, S, GW), bf16),
            pltpu.VMEM((H * HP, S), bf16),
            pltpu.VMEM((1, S), f32),
            pltpu.VMEM((D, S + 256), bf16),
            pltpu.VMEM((D, S), bf16),
            pltpu.VMEM((D, S), f32),
            pltpu.VMEM((S, TQ), f32),
            pltpu.VMEM((S, TQ), f32),
            pltpu.VMEM((S, TQ), f32),
            pltpu.VMEM((H * HP, S), bf16),
        ],
        compiler_params=pltpu.CompilerParams(vmem_limit_bytes=100 * 1024 * 1024),
    )(xt, A_wqkv, A_wo, B_w1, B_w2, B_w3, w4t, gw)
    return out_t.T.reshape(A_x.shape)
```

```python
import contextlib
import math
import os

import jax
import jax.numpy as jnp
from jax import lax
import jax.experimental.pallas as pl
import jax.experimental.pallas.tpu as pltpu

S, D, H, DH, F = 2048, 448, 16, 28, 1792
GW = 4 * DH
HP = 32
TT = 512
TQ = 512
CK = 128
LAG = int(os.environ.get("LAG", 2))
FC = 256
U = int(os.environ.get("U", 9))
PU = int(os.environ.get("PU", 2))
NB = 3
NR = int(os.environ.get("NR", 4))
C4 = D // 4
NT = S // TT
NQ = S // TQ
NSTEP = NQ * H
NC = S // CK
XSPLIT = tuple(int(v) for v in os.environ.get("XS", "0,256,1024,2048").split(","))
FPOS = int(os.environ.get('FPOS', 2))
FSCHED = {
    "a": {1: [(0, 0)], 2: [(1, 0), (0, 1)], 3: [(1, 1), (0, 2)], 4: [(1, 2), (0, 3)], 5: [(1, 3)]},
    "b": {1: [(0, 0)], 2: [(1, 0)], 3: [(0, 1)], 4: [(1, 1)], 5: [(0, 2)], 6: [(1, 2)], 7: [(0, 3)], 8: [(1, 3)]},
    "c": {2: [(0, 0), (0, 1), (1, 0), (0, 2), (1, 1), (0, 3), (1, 2)], 3: [(1, 3)]},
}[os.environ.get('FS', 'b')]
CATCH = int(os.environ.get('CATCH', 12))
SCOPES = os.environ.get("SCOPES") == "1"

bf16 = jnp.bfloat16
f32 = jnp.float32
u32 = jnp.uint32
TN = (((0,), (0,)), ((), ()))


def scope(name):
    return jax.named_scope(name) if SCOPES else contextlib.nullcontext()


def _gelu(x):
    c0 = math.sqrt(2.0 / math.pi)
    inner = x * (c0 + (c0 * 0.044715) * (x * x))
    hx = 0.5 * x
    return hx + hx * jnp.tanh(inner)


def _ln_t(x):
    m = jnp.sum(x, axis=0, keepdims=True) * (1.0 / D)
    xc = x - m
    v = jnp.sum(xc * xc, axis=0, keepdims=True) * (1.0 / D)
    return xc * lax.rsqrt(v + 1e-5)


def _pk(x):
    return pltpu.bitcast(x.astype(bf16), u32)


def _up(x):
    return pltpu.bitcast(x, bf16)


def _dot(a, b):
    return jnp.dot(a, b, preferred_element_type=f32)


def _dot_tn(a, b):
    return lax.dot_general(a, b, TN, preferred_element_type=f32)


def _kernel(xt_hbm, wqkv_hbm, wo_hbm, w1_hbm, w2_hbm, w3_hbm, w4t_hbm, gw_hbm, out_hbm,
            xt_v, wqkv_v, wo_v, w1_v, w2_v, w3_v, w4t_v, gw_v, out_v, sems, out_sem, bar_sem,
            w1t_s, wvt_s, wqkt_s, w2t_s, w3t_s, w4p_s, g_s, wot_s, gw_s,
            xp_s, qt_s, k_s, vt_s, z_s, h_s, ln_s, b_s, s0_s, s1_s, s2_s, ot_s):
    def cp(src, dst, n):
        return pltpu.make_async_copy(src, dst, sems.at[n])

    def cpx(i, n):
        return cp(xt_hbm.at[:, XSPLIT[i]:XSPLIT[i + 1]], xt_v.at[:, XSPLIT[i]:XSPLIT[i + 1]], n)

    cp_x0 = cpx(0, 0)
    cp_w1 = cp(w1_hbm, w1_v, 1)
    cp_wv = cp(wqkv_hbm.at[:, 2 * D:3 * D], wqkv_v.at[:, 2 * D:3 * D], 2)
    cp_gw = cp(gw_hbm, gw_v, 2)
    cp_x1 = cpx(1, 0)
    cp_x2 = cpx(2, 1)
    cp_wqk = cp(wqkv_hbm.at[:, 0:2 * D], wqkv_v.at[:, 0:2 * D], 1)
    cp_w2 = cp(w2_hbm, w2_v, 1)
    cp_wo = cp(wo_hbm, wo_v, 2)
    cp_w3 = cp(w3_hbm, w3_v, 0)
    cp_w4 = cp(w4t_hbm, w4t_v, 0)

    def fence():
        pl.semaphore_signal(bar_sem, 1)
        pl.semaphore_wait(bar_sem, 1)

    cp_x0.start()
    fence()
    cp_w1.start()
    fence()
    cp_wv.start()
    cp_gw.start()

    qscale = (DH ** -0.5) * math.log2(math.e)
    HW = HP // 2

    def span(c0, w):
        return slice(c0, c0 + w) if isinstance(c0, int) else pl.ds(pl.multiple_of(c0, 128), w)

    def gate_logit(c0, w, xf):
        gwc = gw_s[...]
        z_s[:, span(c0, w)] = jnp.sum(xf * jnp.concatenate([gwc] * (w // 128), axis=1), axis=0, keepdims=True)

    def ln1(c0, w, gate=True):
        xf = xt_v[:, span(c0, w)].astype(f32)
        return _ln_t(xf).astype(bf16)

    def mix1(c0, w, ln, w1t):
        h_s[:, span(c0 + 128, w)] = _pk(_gelu(_dot(w1t, ln)))

    def vproj(c0, w, wvt):
        xt = xt_v[:, span(c0, w)]
        xp_s[:, span(c0, w)] = _pk(xt)
        vt = _dot(wvt, xt)
        rid = lax.broadcasted_iota(jnp.int32, (HP - DH, w), 0)
        tail = jnp.where(rid == 0, 1.0, 0.0).astype(f32)
        for h in range(H):
            vt_s[HW * h:HW * (h + 1), span(c0, w)] = _pk(
                jnp.concatenate([vt[DH * h:DH * (h + 1), :], tail], axis=0))

    def pieces(a, b):
        out = []
        while a < b:
            e = min((a // TT + 1) * TT, b)
            out.append((a, e - a))
            a = e
        return out

    h_s[:, 0:128] = jnp.zeros((D // 2, 128), u32)
    h_s[:, S + 128:S + 256] = jnp.zeros((D // 2, 128), u32)
    for sb in (s1_s, s2_s):
        sb[0:8, :] = jnp.zeros((8, TQ), f32)
    for sb in (w3t_s, w4p_s, g_s):
        sb[0:8, 0:128] = jnp.zeros((8, 128), u32)
    with scope("w_x0"):
        cp_x0.wait()
    cp_x1.start()
    ln_s[:, XSPLIT[0]:XSPLIT[1]] = _pk(ln1(XSPLIT[0], XSPLIT[1], gate=False))
    with scope("w_w1"):
        cp_w1.wait()
    w1t = w1_v[...].T
    w1t_s[...] = _pk(w1t)
    mix1(XSPLIT[0], XSPLIT[1], _up(ln_s[:, XSPLIT[0]:XSPLIT[1]]), w1t)
    with scope("w_wv"):
        cp_wv.wait()
        cp_gw.wait()
    cp_x2.start()
    wvt = wqkv_v[:, 2 * D:3 * D].T
    wvt_s[...] = _pk(wvt)
    vproj(XSPLIT[0], XSPLIT[1], wvt)
    gw_s[...] = jnp.broadcast_to(gw_v[...].astype(f32).reshape(1, D), (128, D)).T
    with scope("w_x1"):
        cp_x1.wait()
    cp_wqk.start()
    cp_w2.start()
    cp_wo.start()
    for c0, c1 in pieces(XSPLIT[1], XSPLIT[2]):
        vproj(c0, c1, _up(wvt_s[...]))
        mix1(c0, c1, ln1(c0, c1), _up(w1t_s[...]))
    with scope("w_x2"):
        cp_x2.wait()
        cp_wqk.wait()
        cp_w2.wait()
    cp_w3.start()
    cp_w4.start()
    wqkt_s[...] = _pk(wqkv_v[:, 0:2 * D].T)
    w2t_s[...] = _pk(w2_v[...].T)
    for c0, c1 in pieces(XSPLIT[2], XSPLIT[3]):
        vproj(c0, c1, _up(wvt_s[...]))
        mix1(c0, c1, ln1(c0, c1), _up(w1t_s[...]))
    with scope("w_w2"):
        cp_wo.wait()

    def proj(i, m):
        t0 = pl.multiple_of(i * TT, TT)
        cols = pl.ds(t0, TT)
        xt = _up(xp_s[:, cols])
        zpad = jnp.zeros((HP - DH, TT), f32)

        def heads(y, n):
            return [jnp.concatenate([y[DH * h:DH * (h + 1), :], zpad], axis=0).astype(bf16) for h in range(n)]

        kn = [kh.T for kh in heads(_dot(_up(wqkt_s[D // 2:D, :]), xt), H)]
        for h in range(H):
            k_s[h, pl.ds(pl.multiple_of(i * (TT // 2), TT // 2), TT // 2), :] = _pk(kn[h])
        hw = h_s[:, pl.ds(t0, TT + 256)]
        c8 = C4 // 2
        hs = _up(jnp.concatenate([
            hw[0 * c8:1 * c8, 127:127 + TT],
            hw[1 * c8:2 * c8, 129:129 + TT],
            hw[2 * c8:3 * c8, 126:126 + TT],
            hw[3 * c8:4 * c8, 130:130 + TT]], axis=0))
        for h, qh in enumerate(heads(_dot(_up(wqkt_s[0:GW // 2, :]), xt) * qscale, 4)):
            qt_s[HW * h:HW * (h + 1), cols] = _pk(qh)
        x1 = xt.astype(f32) + _dot(_up(w2t_s[...]), hs)
        b_s[:, cols] = x1
        ln_s[:, cols] = _pk(_ln_t(x1))
        s = _dot(kn[0], _up(qt_s[0:HW, 0:TQ]))
        s0_s[cols, :] = s
        m = jnp.maximum(m, jnp.max(s.reshape(TT // 8, 8, TQ), axis=0))
        for h, qh in enumerate(heads(_dot(_up(wqkt_s[GW // 2:D // 2, :]), xt) * qscale, H - 4)):
            qt_s[HW * (h + 4):HW * (h + 5), cols] = _pk(qh)
        wo_f = wo_v[pl.ds(pl.multiple_of(i * GW, 16), GW), :].astype(f32)
        zrows = jnp.zeros((HP - DH, D), f32)
        parts = []
        for j in range(4):
            parts += [wo_f[DH * j:DH * (j + 1), :], zrows]
        wot_s[:, pl.ds(pl.multiple_of(i * 128, 128), 128)] = _pk(jnp.concatenate(parts, axis=0).astype(bf16).T)
        return m

    def proj_body(ii, m):
        for u in range(PU):
            m = proj(ii * PU + u, m)
        return m

    with scope("proj"):
        m = lax.fori_loop(0, NT // PU, proj_body, jnp.full((8, TQ), -jnp.inf, f32))

    cp_w3.wait()
    cp_w4.wait()

    sbuf = (s0_s, s1_s, s2_s)

    def body(i, m_in):
        fcols = pl.ds(pl.multiple_of(i * FC, FC), FC)
        w3t_s[...] = _pk(w3_v[:, fcols].T)
        w4p_s[...] = _pk(w4t_v[:, fcols])

        def ffn_up(tb):
            cols = slice(tb * TT, (tb + 1) * TT)
            g_s[:, cols] = _pk(_gelu(_dot(_up(w3t_s[...]), _up(ln_s[:, cols]))))

        def ffn_down(tb):
            cols = slice(tb * TT, (tb + 1) * TT)
            b_s[:, cols] += _dot(_up(w4p_s[...]), _up(g_s[:, cols]))

        ntot = U * NC
        order = []
        done = 0
        for n in range(ntot):
            if n >= ntot - CATCH:
                k = n - (ntot - CATCH) + 1
                target = n - LAG + (k * (LAG + 1) + CATCH - 1) // CATCH
                target = min(target, ntot)
                while done < target:
                    order.append((1, done))
                    done += 1
                order.append((0, n))
            else:
                order.append((0, n))
                while done <= n - LAG:
                    order.append((1, done))
                    done += 1
        assert done == ntot
        mx = {-1: m_in}
        mrow = {}
        qms = {}
        accs = {}
        for kind, n in order:
            u, cc = divmod(n, NC)
            if kind == 0 and cc == FPOS and u >= 1:
                for typ, tb in FSCHED.get(u, ()):
                    (ffn_up if typ == 0 else ffn_down)(tb)
            ks = slice(cc * CK, (cc + 1) * CK)
            if kind == 0:
                t1 = i * U + u + 1
                h1 = t1 & (H - 1)
                if cc == 0:
                    qms[u] = _up(qt_s[pl.ds(pl.multiple_of(h1 * HW, HW), HW),
                                      pl.ds(pl.multiple_of((t1 >> 4) * TQ, TQ), TQ)])
                s = _dot(_up(k_s[h1, cc * CK // 2:(cc + 1) * CK // 2, :]), qms[u])
                sbuf[(u + 1) % NB][ks, :] = s
                mc = jnp.max(s.reshape(CK // 8, 8, TQ), axis=0)
                mx[u] = mc if cc == 0 else jnp.maximum(mx[u], mc)
            else:
                t2 = i * U + u
                hrows = pl.ds(pl.multiple_of((t2 & (H - 1)) * HW, HW), HW)
                if cc == 0:
                    mrow[u] = jnp.max(mx[u - 1], axis=0, keepdims=True)
                p = jnp.exp2(sbuf[u % NB][ks, :] - mrow[u]).astype(bf16)
                pv = _dot(_up(vt_s[hrows, ks]), p)
                accs[u] = pv if cc == 0 else accs[u] + pv
                if cc == NC - 1:
                    acc = accs[u]
                    inv = 1.0 / acc[DH:DH + 1, :]
                    ot_s[hrows, pl.ds(pl.multiple_of((t2 >> 4) * TQ, TQ), TQ)] = _pk(acc * inv)
        return mx[U - 1]

    with scope("attn"):
        m = lax.fori_loop(0, (NSTEP - 1) // U, body, m)

    s_last = sbuf[(NSTEP - 1) % NB]
    RP = D // NR
    m_last = jnp.max(m, axis=0, keepdims=True)
    pacc = None
    npv = 0
    nslots = (NT - 1) * NR - 2
    with scope("tail"):
        for tb in range(NT):
            cols = slice(tb * TT, (tb + 1) * TT)
            gwc = gw_s[...]
            z = jnp.sum(_up(xp_s[:, cols]).astype(f32) * jnp.concatenate([gwc] * (TT // 128), axis=1),
                        axis=0, keepdims=True)
            gate = 1.0 / (1.0 + jnp.exp(-z))
            ot = _up(ot_s[:, cols])
            for r in range(NR):
                rows = slice(r * RP, (r + 1) * RP)
                a = _dot(_up(wot_s[r * RP // 2:(r + 1) * RP // 2, :]), ot)
                bb = b_s[rows, cols]
                out_v[rows, cols] = (bb + gate * (a - bb)).astype(bf16)
                if tb == NT - 1:
                    pltpu.make_async_copy(out_v.at[rows, cols], out_hbm.at[rows, cols], out_sem).start()
                slot = tb * NR + r + 1
                while npv < NC and npv * nslots < slot * NC:
                    ks = slice(npv * CK, (npv + 1) * CK)
                    p = jnp.exp2(s_last[ks, :] - m_last).astype(bf16)
                    pv = _dot(_up(vt_s[(H - 1) * HW:H * HW, ks]), p)
                    pacc = pv if pacc is None else pacc + pv
                    npv += 1
                    if npv == NC:
                        inv = 1.0 / pacc[DH:DH + 1, :]
                        ot_s[(H - 1) * HW:H * HW, S - TQ:S] = _pk(pacc * inv)
            if tb < NT - 1:
                pltpu.make_async_copy(out_v.at[:, cols], out_hbm.at[:, cols], out_sem).start()
    with scope("w_out"):
        pltpu.make_async_copy(out_v, out_hbm, out_sem).wait()


@jax.jit
def pallas_gated_mix__mha_block__mixer_s_mlp__prompt_kernel(A_x, A_wqkv, A_wo, B_x, B_w1, B_w2, B_w3, B_w4, gate_w):
    xt = A_x.reshape(S, D).T
    w4t = B_w4.T
    any_spec = pl.BlockSpec(memory_space=pl.ANY)
    out_t = pl.pallas_call(
        _kernel,
        out_shape=jax.ShapeDtypeStruct((D, S), A_x.dtype),
        in_specs=[any_spec] * 8,
        out_specs=any_spec,
        scratch_shapes=[
            pltpu.VMEM((D, S), bf16),
            pltpu.VMEM((D, 3 * D), bf16),
            pltpu.VMEM((D, D), bf16),
            pltpu.VMEM((D, D), bf16),
            pltpu.VMEM((D, D), bf16),
            pltpu.VMEM((D, F), bf16),
            pltpu.VMEM((D, F), bf16),
            pltpu.VMEM((D,), bf16),
            pltpu.VMEM((D, S), bf16),
            pltpu.SemaphoreType.DMA((3,)),
            pltpu.SemaphoreType.DMA(()),
            pltpu.SemaphoreType.REGULAR,
            pltpu.VMEM((D // 2, D), u32),
            pltpu.VMEM((D // 2, D), u32),
            pltpu.VMEM((D, D), u32),
            pltpu.VMEM((D // 2, D), u32),
            pltpu.VMEM((FC // 2, D), u32),
            pltpu.VMEM((D // 2, FC), u32),
            pltpu.VMEM((FC // 2, S), u32),
            pltpu.VMEM((D // 2, H * HP), u32),
            pltpu.VMEM((D, 128), f32),
            pltpu.VMEM((D // 2, S), u32),
            pltpu.VMEM((H * HP // 2, S), u32),
            pltpu.VMEM((H, S // 2, HP), u32),
            pltpu.VMEM((H * HP // 2, S), u32),
            pltpu.VMEM((1, S), f32),
            pltpu.VMEM((D // 2, S + 256), u32),
            pltpu.VMEM((D // 2, S), u32),
            pltpu.VMEM((D, S), f32),
            pltpu.VMEM((S, TQ), f32),
            pltpu.VMEM((S, TQ), f32),
            pltpu.VMEM((S, TQ), f32),
            pltpu.VMEM((H * HP // 2, S), u32),
        ],
        compiler_params=pltpu.CompilerParams(vmem_limit_bytes=100 * 1024 * 1024),
    )(xt, A_wqkv, A_wo, B_w1, B_w2, B_w3, w4t, gate_w)
    return out_t.T.reshape(A_x.shape)
```

```python
import math

import jax
import jax.numpy as jnp
from jax import lax
import jax.experimental.pallas as pl
import jax.experimental.pallas.tpu as pltpu

S, D, H, DH, F = 2048, 448, 16, 28, 1792
GW = 4 * DH
HP = 32
HW = HP // 2
TT = 512
TQ = 512
CK = 128
LAG = 2
CATCH = 12
FC = 256
U = 9
PU = 2
NB = 3
NR = 4
C4 = D // 4
D2, F2, T2 = D // 2, FC // 2, TT // 2
NT = S // TT
NSTEP = (S // TQ) * H
NC = S // CK
XSPLIT = (0, 256, 1024, 2048)
KSPLIT = ((0, 256), (256, D))

bf16 = jnp.bfloat16
f32 = jnp.float32
u32 = jnp.uint32

_LHS = ((0, 3, 1), (2, 3, 1), (0, None, 0), (3, None, 0), (0, 1, 1), (2, 0, -1), (1, 3, -1))
_RHS = ((0, 3, 1), (0, None, 0), (1, 3, -1), (2, 0, -1), (3, None, 0), (0, 1, 1), (2, 3, 1))


def _gelu(x):
    c0 = math.sqrt(2.0 / math.pi)
    inner = x * (c0 + (c0 * 0.044715) * (x * x))
    hx = 0.5 * x
    return hx + hx * jnp.tanh(inner)


def _ln_t(x):
    m = jnp.sum(x, axis=0, keepdims=True) * (1.0 / D)
    xc = x - m
    v = jnp.sum(xc * xc, axis=0, keepdims=True) * (1.0 / D)
    return xc * lax.rsqrt(v + 1e-5)


def _pk(x):
    return pltpu.bitcast(x.astype(bf16), u32)


def _up(x):
    return pltpu.bitcast(x, bf16)


def _dot(a, b):
    return jnp.dot(a, b, preferred_element_type=f32)


def _operand(term, quad):
    a, b, sign = term
    if sign == 0:
        return quad(a).astype(bf16)
    ta, tb = quad(a).astype(f32), quad(b).astype(f32)
    return (ta + tb if sign > 0 else ta - tb).astype(bf16)


def _span(c0, w, align=128):
    return slice(c0, c0 + w) if isinstance(c0, int) else pl.ds(pl.multiple_of(c0, align), w)


def _chunk_order():
    ntot = U * NC
    order = []
    done = 0
    for n in range(ntot):
        if n >= ntot - CATCH:
            k = n - (ntot - CATCH) + 1
            target = min(n - LAG + (k * (LAG + 1) + CATCH - 1) // CATCH, ntot)
            while done < target:
                order.append((1, done))
                done += 1
            order.append((0, n))
        else:
            order.append((0, n))
            while done <= n - LAG:
                order.append((1, done))
                done += 1
    assert done == ntot
    return order


def _kernel(xt_hbm, wqkv_hbm, wo_hbm, w1_hbm, w2_hbm, w3_hbm, w4t_hbm, gw_hbm, out_hbm,
            xt_v, wqkv_v, wo_v, w1_v, w2_v, w3_v, w4t_v, gw_v, out_v, sems, out_sem, bar_sem,
            w1t_s, wvt_s, wqkt_s, w2t_s, w3k_s, w4k_s, wot_s, gw_s,
            g_s, macc_s, st_s, lnf_s, b_s,
            xp_s, qt_s, k_s, vt_s, h_s, s0_s, s1_s, s2_s, ot_s, ln0_s):
    def cp(src, dst, n):
        return pltpu.make_async_copy(src, dst, sems.at[n])

    def cpx(i, n):
        return cp(xt_hbm.at[:, XSPLIT[i]:XSPLIT[i + 1]], xt_v.at[:, XSPLIT[i]:XSPLIT[i + 1]], n)

    cp_x0 = cpx(0, 0)
    cp_w1 = cp(w1_hbm, w1_v, 1)
    cp_wv = cp(wqkv_hbm.at[:, 2 * D:3 * D], wqkv_v.at[:, 2 * D:3 * D], 2)
    cp_gw = cp(gw_hbm, gw_v, 2)
    cp_x1 = cpx(1, 0)
    cp_x2 = cpx(2, 1)
    cp_wqk = cp(wqkv_hbm.at[:, 0:2 * D], wqkv_v.at[:, 0:2 * D], 1)
    cp_w2 = cp(w2_hbm, w2_v, 1)
    cp_w3a = cp(w3_hbm.at[:, 0:FC], w3_v.at[:, 0:FC], 1)
    cp_w4a = cp(w4t_hbm.at[:, 0:FC], w4t_v.at[:, 0:FC], 1)
    cp_wo = cp(wo_hbm, wo_v, 2)
    cp_w3 = cp(w3_hbm.at[:, FC:F], w3_v.at[:, FC:F], 0)
    cp_w4 = cp(w4t_hbm.at[:, FC:F], w4t_v.at[:, FC:F], 0)

    def fence():
        pl.semaphore_signal(bar_sem, 1)
        pl.semaphore_wait(bar_sem, 1)

    cp_x0.start()
    fence()
    cp_w1.start()
    fence()
    cp_wv.start()
    cp_gw.start()

    qscale = (DH ** -0.5) * math.log2(math.e)

    def ln1(c0, w):
        return _ln_t(xt_v[:, c0:c0 + w].astype(f32))

    def put_h(c0, y):
        h_s[:, c0 + 128:c0 + 128 + y.shape[1]] = _pk(_gelu(y))

    def put_v(c0, y):
        w = y.shape[1]
        rid = lax.broadcasted_iota(jnp.int32, (HP - DH, w), 0)
        tail = jnp.where(rid == 0, 1.0, 0.0).astype(f32)
        for h in range(H):
            vt_s[HW * h:HW * (h + 1), c0:c0 + w] = _pk(
                jnp.concatenate([y[DH * h:DH * (h + 1), :], tail], axis=0))

    def first_use(w_ref, c0, wt_ref, rhs):
        y = None
        for k0, k1 in KSPLIT:
            wt = w_ref[k0:k1, c0:c0 + D].T
            wt_ref[:, k0:k1] = _pk(wt)
            part = _dot(wt, rhs[k0:k1, :])
            y = part if y is None else y + part
        return y

    def ffn_prep(c):
        for k in range(7):
            w3k_s[k] = _pk(_operand(_LHS[k], lambda q: w3_v[(q % 2) * D2:(q % 2 + 1) * D2,
                                                            _span(c * FC + (q // 2) * F2, F2)]).T)
            w4k_s[k] = _pk(_operand(_LHS[k], lambda q: w4t_v[(q // 2) * D2:(q // 2 + 1) * D2,
                                                             _span(c * FC + (q % 2) * F2, F2)]))

    def stage_a(c0, w):
        xt = xt_v[:, c0:c0 + w]
        xp_s[:, c0:c0 + w] = _pk(xt)
        put_v(c0, _dot(_up(wvt_s[...]), xt))
        put_h(c0, _dot(_up(w1t_s[...]), ln1(c0, w).astype(bf16)))

    h_s[:, 0:128] = jnp.zeros((D2, 128), u32)
    h_s[:, S + 128:S + 256] = jnp.zeros((D2, 128), u32)
    for sb in (s1_s, s2_s):
        sb[0:8, :] = jnp.zeros((8, TQ), f32)
    g_s[0, 0:8, 0:128] = jnp.zeros((8, 128), f32)
    st_s[0, 0, 0:8, 0:128] = jnp.zeros((8, 128), f32)
    for k in (0, 1, 2, 3):
        macc_s[k] = jnp.zeros(macc_s.shape[1:], f32)
    w0 = XSPLIT[1]
    cp_x0.wait()
    cp_x1.start()
    macc_s[4] = jnp.zeros(macc_s.shape[1:], f32)
    ln0_s[...] = _pk(ln1(0, w0))
    cp_w1.wait()
    put_h(0, first_use(w1_v, 0, w1t_s, _up(ln0_s[...])))
    cp_wv.wait()
    cp_gw.wait()
    cp_x2.start()
    put_v(0, first_use(wqkv_v, 2 * D, wvt_s, xt_v[:, 0:w0]))
    xp_s[:, 0:w0] = _pk(xt_v[:, 0:w0])
    gw_s[...] = jnp.broadcast_to(gw_v[...].astype(f32).reshape(1, D), (128, D)).T
    cp_x1.wait()
    cp_wqk.start()
    cp_w2.start()
    cp_w3a.start()
    cp_w4a.start()
    stage_a(256, 256)
    stage_a(512, 512)
    cp_x2.wait()
    cp_wqk.wait()
    cp_w2.wait()
    cp_w3a.wait()
    cp_w4a.wait()
    cp_wo.start()
    fence()
    cp_w3.start()
    cp_w4.start()
    ffn_prep(0)
    wqkt_s[...] = _pk(wqkv_v[:, 0:2 * D].T)
    w2t_s[...] = _pk(w2_v[...].T)
    stage_a(1024, 512)
    stage_a(1536, 512)
    cp_wo.wait()

    def proj(i, m):
        cols = _span(i * TT, TT)
        xt = _up(xp_s[:, cols])
        zpad = jnp.zeros((HP - DH, TT), f32)

        def heads(y, n):
            return [jnp.concatenate([y[DH * h:DH * (h + 1), :], zpad], axis=0).astype(bf16) for h in range(n)]

        kn = [kh.T for kh in heads(_dot(_up(wqkt_s[D2:D, :]), xt), H)]
        for h in range(H):
            k_s[h, _span(i * T2, T2), :] = _pk(kn[h])
        hw = h_s[:, _span(i * TT, TT + 256)]
        c8 = C4 // 2
        hs = _up(jnp.concatenate([
            hw[0 * c8:1 * c8, 127:127 + TT],
            hw[1 * c8:2 * c8, 129:129 + TT],
            hw[2 * c8:3 * c8, 126:126 + TT],
            hw[3 * c8:4 * c8, 130:130 + TT]], axis=0))

        def qproj(h0, h1):
            y = _dot(_up(wqkt_s[h0 * DH // 2:h1 * DH // 2, :]), xt) * qscale
            for h, qh in enumerate(heads(y, h1 - h0)):
                qt_s[HW * (h + h0):HW * (h + h0 + 1), cols] = _pk(qh)

        qproj(0, 4)
        x1 = xt.astype(f32) + _dot(_up(w2t_s[...]), hs)
        hcols = _span(i * T2, T2)
        macc_s[6, :, hcols] = x1[0:D2, 0:T2]
        b_s[0, :, hcols] = x1[0:D2, T2:TT]
        b_s[1, :, hcols] = x1[D2:D, 0:T2]
        macc_s[5, :, hcols] = x1[D2:D, T2:TT]
        lnf_s[:, cols] = _ln_t(x1)
        s = _dot(kn[0], _up(qt_s[0:HW, 0:TQ]))
        s0_s[cols, :] = s
        m = jnp.maximum(m, jnp.max(s.reshape(TT // 8, 8, TQ), axis=0))
        qproj(4, H)
        wo_f = wo_v[_span(i * GW, GW, 16), :].astype(f32)
        zrows = jnp.zeros((HP - DH, D), f32)
        parts = []
        for j in range(4):
            parts += [wo_f[DH * j:DH * (j + 1), :], zrows]
        wot_s[:, _span(i * 128, 128)] = _pk(jnp.concatenate(parts, axis=0).astype(bf16).T)
        return m

    def proj_body(ii, m):
        for u in range(PU):
            m = proj(ii * PU + u, m)
        return m

    m = lax.fori_loop(0, NT // PU, proj_body, jnp.full((8, TQ), -jnp.inf, f32))
    cp_w3.wait()
    cp_w4.wait()

    sbuf = (s0_s, s1_s, s2_s)

    def ffn_up(tb):
        def prod(k):
            return _dot(_up(w3k_s[k]), _operand(
                _RHS[k], lambda q: lnf_s[(q // 2) * D2:(q // 2 + 1) * D2,
                                         tb * TT + (q % 2) * T2:tb * TT + (q % 2 + 1) * T2]))

        def emit(q, c):
            g_s[q, :, tb * T2:(tb + 1) * T2] = _gelu(c)

        st = st_s.at[tb % 2]
        st[0] = prod(2)
        m5 = prod(4)
        emit(1, st[0] + m5)
        st[2] = m5
        m2 = prod(1)
        st[3] = st[0] - m2
        st[1] = m2
        m4 = prod(3)
        emit(2, st[1] + m4)
        st[2] = m4 - st[2]
        st[0] = prod(0)
        emit(0, st[2] + st[0] + prod(6))
        emit(3, st[3] + st[0] + prod(5))

    def ffn_down(p):
        cols = slice(p * TT, (p + 1) * TT)
        for k in (1, 3, 5, 0, 2, 4, 6):
            macc_s[k, :, cols] += _dot(_up(w4k_s[k]), _operand(_RHS[k], lambda q: g_s[q, :, cols]))

    def body(i, m_in):
        extra = {1: lambda: ffn_up(0), 2: lambda: ffn_up(1), 3: lambda: ffn_up(2), 4: lambda: ffn_down(0),
                 5: lambda: ffn_up(3), 6: lambda: ffn_down(1),
                 7: lambda: ffn_prep(jnp.minimum(i + 1, F // FC - 1))}
        mx = {-1: m_in}
        mrow = {}
        qms = {}
        accs = {}
        for kind, n in _chunk_order():
            u, cc = divmod(n, NC)
            if kind == 0 and cc == LAG and u in extra:
                extra[u]()
            ks = slice(cc * CK, (cc + 1) * CK)
            if kind == 0:
                t1 = i * U + u + 1
                h1 = t1 & (H - 1)
                if cc == 0:
                    qms[u] = _up(qt_s[_span(h1 * HW, HW, HW), _span((t1 >> 4) * TQ, TQ)])
                s = _dot(_up(k_s[h1, cc * CK // 2:(cc + 1) * CK // 2, :]), qms[u])
                sbuf[(u + 1) % NB][ks, :] = s
                mc = jnp.max(s.reshape(CK // 8, 8, TQ), axis=0)
                mx[u] = mc if cc == 0 else jnp.maximum(mx[u], mc)
            else:
                t2 = i * U + u
                hrows = _span((t2 & (H - 1)) * HW, HW, HW)
                if cc == 0:
                    mrow[u] = jnp.max(mx[u - 1], axis=0, keepdims=True)
                p = jnp.exp2(sbuf[u % NB][ks, :] - mrow[u]).astype(bf16)
                pv = _dot(_up(vt_s[hrows, ks]), p)
                accs[u] = pv if cc == 0 else accs[u] + pv
                if cc == NC - 1:
                    acc = accs[u]
                    inv = 1.0 / acc[DH:DH + 1, :]
                    ot_s[hrows, _span((t2 >> 4) * TQ, TQ)] = _pk(acc * inv)
        return mx[U - 1]

    m = lax.fori_loop(0, (NSTEP - 1) // U, body, m)

    s_last = sbuf[(NSTEP - 1) % NB]
    m_last = jnp.max(m, axis=0, keepdims=True)

    def last_pv():
        pacc = None
        for cc in range(NC):
            ks = slice(cc * CK, (cc + 1) * CK)
            p = jnp.exp2(s_last[ks, :] - m_last).astype(bf16)
            pv = _dot(_up(vt_s[(H - 1) * HW:H * HW, ks]), p)
            pacc = pv if pacc is None else pacc + pv
            if cc == NC - 1:
                inv = 1.0 / pacc[DH:DH + 1, :]
                ot_s[(H - 1) * HW:H * HW, S - TQ:S] = _pk(pacc * inv)
            yield

    def mixer_out(q, rows, hc):
        def mk(k):
            return macc_s[k, rows, hc]

        if q == 0:
            return mk(0) + mk(3) - mk(4) + mk(6)
        if q == 1:
            return mk(2) + mk(4) + b_s[0, rows, hc]
        if q == 2:
            return mk(1) + mk(3) + b_s[1, rows, hc]
        return mk(0) - mk(1) + mk(2) + mk(5)

    pvs = last_pv()
    nslots = (NT - 1) * NR - 2
    npv = 0
    RP = D // NR
    for tb in range(NT):
        cols = slice(tb * TT, (tb + 1) * TT)
        hc = slice(tb * T2, (tb + 1) * T2)
        gwc = gw_s[...]
        z = jnp.sum(_up(xp_s[:, cols]).astype(f32) * jnp.concatenate([gwc] * (TT // 128), axis=1),
                    axis=0, keepdims=True)
        gate = 1.0 / (1.0 + jnp.exp(-z))
        ot = _up(ot_s[:, cols])
        for r in range(NR):
            rows = slice(r * RP, (r + 1) * RP)
            a = _dot(_up(wot_s[r * RP // 2:(r + 1) * RP // 2, :]), ot)
            half, r0 = divmod(r * RP, D2)
            rr = slice(r0, r0 + RP)
            bb = jnp.concatenate([mixer_out(2 * half, rr, hc), mixer_out(2 * half + 1, rr, hc)], axis=1)
            out_v[rows, cols] = (bb + gate * (a - bb)).astype(bf16)
            pltpu.make_async_copy(out_v.at[rows, cols], out_hbm.at[rows, cols], out_sem).start()
            while npv < NC and npv * nslots < (tb * NR + r + 1) * NC:
                next(pvs)
                npv += 1
    pltpu.make_async_copy(out_v, out_hbm, out_sem).wait()


@jax.jit
def pallas_gated_mix__mha_block__mixer_s_mlp__prompt_kernel(
    A_x: jax.Array,
    A_wqkv: jax.Array,
    A_wo: jax.Array,
    B_x: jax.Array,
    B_w1: jax.Array,
    B_w2: jax.Array,
    B_w3: jax.Array,
    B_w4: jax.Array,
    gate_w: jax.Array,
):
    del B_x
    any_spec = pl.BlockSpec(memory_space=pl.ANY)
    out_t = pl.pallas_call(
        _kernel,
        out_shape=jax.ShapeDtypeStruct((D, S), A_x.dtype),
        in_specs=[any_spec] * 8,
        out_specs=any_spec,
        scratch_shapes=[
            pltpu.VMEM((D, S), bf16),
            pltpu.VMEM((D, 3 * D), bf16),
            pltpu.VMEM((D, D), bf16),
            pltpu.VMEM((D, D), bf16),
            pltpu.VMEM((D, D), bf16),
            pltpu.VMEM((D, F), bf16),
            pltpu.VMEM((D, F), bf16),
            pltpu.VMEM((D,), bf16),
            pltpu.VMEM((D, S), bf16),
            pltpu.SemaphoreType.DMA((3,)),
            pltpu.SemaphoreType.DMA(()),
            pltpu.SemaphoreType.REGULAR,
            pltpu.VMEM((D2, D), u32),
            pltpu.VMEM((D2, D), u32),
            pltpu.VMEM((D, D), u32),
            pltpu.VMEM((D2, D), u32),
            pltpu.VMEM((7, F2 // 2, D2), u32),
            pltpu.VMEM((7, D2 // 2, F2), u32),
            pltpu.VMEM((D2, H * HP), u32),
            pltpu.VMEM((D, 128), f32),
            pltpu.VMEM((4, F2, S // 2), f32),
            pltpu.VMEM((7, D2, S // 2), f32),
            pltpu.VMEM((2, 4, F2, T2), f32),
            pltpu.VMEM((D, S), f32),
            pltpu.VMEM((2, D2, S // 2), f32),
            pltpu.VMEM((D2, S), u32),
            pltpu.VMEM((H * HW, S), u32),
            pltpu.VMEM((H, S // 2, HP), u32),
            pltpu.VMEM((H * HW, S), u32),
            pltpu.VMEM((D2, S + 256), u32),
            pltpu.VMEM((S, TQ), f32),
            pltpu.VMEM((S, TQ), f32),
            pltpu.VMEM((S, TQ), f32),
            pltpu.VMEM((H * HW, S), u32),
            pltpu.VMEM((D2, XSPLIT[1]), u32),
        ],
        compiler_params=pltpu.CompilerParams(vmem_limit_bytes=100 * 1024 * 1024),
    )(A_x.reshape(S, D).T, A_wqkv, A_wo, B_w1, B_w2, B_w3, B_w4.T, gate_w)
    return out_t.T.reshape(A_x.shape)
```

```python
import math

import jax
import jax.numpy as jnp
from jax import lax
import jax.experimental.pallas as pl
import jax.experimental.pallas.tpu as pltpu

S, D, H, DH, F = 2048, 448, 16, 28, 1792
GW = 4 * DH
HP = 32
HW = HP // 2
TT = 512
TQ = 512
CK = 128
LAG = 2
CATCH = 12
FC = 256
U = 9
PU = 2
NB = 3
NR = 4
C4 = D // 4
D2, F2, T2 = D // 2, FC // 2, TT // 2
NT = S // TT
NSTEP = (S // TQ) * H
NC = S // CK
XSPLIT = (0, 256, 1024, 2048)
KSPLIT = ((0, 256), (256, D))

bf16 = jnp.bfloat16
f32 = jnp.float32
u32 = jnp.uint32

_LHS = ((0, 3, 1), (2, 3, 1), (0, None, 0), (3, None, 0), (0, 1, 1), (2, 0, -1), (1, 3, -1))
_RHS = ((0, 3, 1), (0, None, 0), (1, 3, -1), (2, 0, -1), (3, None, 0), (0, 1, 1), (2, 3, 1))


def _gelu(x):
    c0 = math.sqrt(2.0 / math.pi)
    inner = x * (c0 + (c0 * 0.044715) * (x * x))
    hx = 0.5 * x
    return hx + hx * jnp.tanh(inner)


def _ln_t(x):
    m = jnp.sum(x, axis=0, keepdims=True) * (1.0 / D)
    xc = x - m
    v = jnp.sum(xc * xc, axis=0, keepdims=True) * (1.0 / D)
    return xc * lax.rsqrt(v + 1e-5)


def _pk(x):
    return pltpu.bitcast(x.astype(bf16), u32)


def _up(x):
    return pltpu.bitcast(x, bf16)


def _dot(a, b):
    return jnp.dot(a, b, preferred_element_type=f32)


def _operand(term, quad):
    a, b, sign = term
    if sign == 0:
        return quad(a).astype(bf16)
    ta, tb = quad(a).astype(f32), quad(b).astype(f32)
    return (ta + tb if sign > 0 else ta - tb).astype(bf16)


def _span(c0, w, align=128):
    return slice(c0, c0 + w) if isinstance(c0, int) else pl.ds(pl.multiple_of(c0, align), w)


def _chunk_order():
    ntot = U * NC
    order = []
    done = 0
    for n in range(ntot):
        if n >= ntot - CATCH:
            k = n - (ntot - CATCH) + 1
            target = min(n - LAG + (k * (LAG + 1) + CATCH - 1) // CATCH, ntot)
            while done < target:
                order.append((1, done))
                done += 1
            order.append((0, n))
        else:
            order.append((0, n))
            while done <= n - LAG:
                order.append((1, done))
                done += 1
    assert done == ntot
    return order


def _kernel(xt_hbm, wqkv_hbm, wo_hbm, w1_hbm, w2_hbm, w3_hbm, w4t_hbm, gw_hbm, out_hbm,
            xt_v, wqkv_v, wo_v, w1_v, w2_v, w3_v, w4t_v, gw_v, out_v, sems, out_sem, bar_sem,
            w1t_s, wvt_s, wqkt_s, w2t_s, w3k_s, w4k_s, wot_s, gw_s,
            g_s, macc_s, st_s, lnf_s, b_s,
            xp_s, qt_s, k_s, vt_s, h_s, s0_s, s1_s, s2_s, ot_s, ln0_s, gate_s):
    def cp(src, dst, n):
        return pltpu.make_async_copy(src, dst, sems.at[n])

    def cpx(i, n):
        return cp(xt_hbm.at[:, XSPLIT[i]:XSPLIT[i + 1]], xt_v.at[:, XSPLIT[i]:XSPLIT[i + 1]], n)

    cp_x0 = cpx(0, 0)
    cp_w1 = cp(w1_hbm, w1_v, 1)
    cp_wv = cp(wqkv_hbm.at[:, 2 * D:3 * D], wqkv_v.at[:, 2 * D:3 * D], 2)
    cp_gw = cp(gw_hbm, gw_v, 2)
    cp_x1 = cpx(1, 0)
    cp_x2 = cpx(2, 1)
    cp_wqk = cp(wqkv_hbm.at[:, 0:2 * D], wqkv_v.at[:, 0:2 * D], 1)
    cp_w2 = cp(w2_hbm, w2_v, 1)
    cp_w3a = cp(w3_hbm.at[:, 0:FC], w3_v.at[:, 0:FC], 1)
    cp_wo = cp(wo_hbm, wo_v, 2)
    cp_w3 = cp(w3_hbm.at[:, FC:F], w3_v.at[:, FC:F], 0)
    cp_w4 = cp(w4t_hbm, w4t_v, 0)

    def fence():
        pl.semaphore_signal(bar_sem, 1)
        pl.semaphore_wait(bar_sem, 1)

    cp_x0.start()
    fence()
    cp_w1.start()
    fence()
    cp_wv.start()
    cp_gw.start()

    qscale = (DH ** -0.5) * math.log2(math.e)

    def ln1(c0, w):
        return _ln_t(xt_v[:, c0:c0 + w].astype(f32))

    def put_h(c0, y):
        h_s[:, c0 + 128:c0 + 128 + y.shape[1]] = _pk(_gelu(y))

    def put_v(c0, y):
        w = y.shape[1]
        rid = lax.broadcasted_iota(jnp.int32, (HP - DH, w), 0)
        tail = jnp.where(rid == 0, 1.0, 0.0).astype(f32)
        for h in range(H):
            vt_s[HW * h:HW * (h + 1), c0:c0 + w] = _pk(
                jnp.concatenate([y[DH * h:DH * (h + 1), :], tail], axis=0))

    def first_use(w_ref, c0, wt_ref, rhs):
        y = None
        for k0, k1 in KSPLIT:
            wt = w_ref[k0:k1, c0:c0 + D].T
            wt_ref[:, k0:k1] = _pk(wt)
            part = _dot(wt, rhs[k0:k1, :])
            y = part if y is None else y + part
        return y

    def prep_up(c):
        for k in range(7):
            w3k_s[k] = _pk(_operand(_LHS[k], lambda q: w3_v[(q % 2) * D2:(q % 2 + 1) * D2,
                                                            _span(c * FC + (q // 2) * F2, F2)]).T)

    def prep_down(c):
        for k in range(7):
            w4k_s[k] = _pk(_operand(_LHS[k], lambda q: w4t_v[(q // 2) * D2:(q // 2 + 1) * D2,
                                                             _span(c * FC + (q % 2) * F2, F2)]))

    def stage_v(c0, w):
        xt = xt_v[:, c0:c0 + w]
        xp_s[:, c0:c0 + w] = _pk(xt)
        put_v(c0, _dot(_up(wvt_s[...]), xt))

    def stage_h(c0, w):
        put_h(c0, _dot(_up(w1t_s[...]), ln1(c0, w).astype(bf16)))

    def gate_of(x):
        gwc = gw_s[...]
        z = jnp.sum(x.astype(f32) * jnp.concatenate([gwc] * (TT // 128), axis=1), axis=0, keepdims=True)
        return 1.0 / (1.0 + jnp.exp(-z))

    h_s[:, 0:128] = jnp.zeros((D2, 128), u32)
    h_s[:, S + 128:S + 256] = jnp.zeros((D2, 128), u32)
    for sb in (s1_s, s2_s):
        sb[0:8, :] = jnp.zeros((8, TQ), f32)
    g_s[0, 0:8, 0:128] = jnp.zeros((8, 128), f32)
    w4k_s[0, 0:8, 0:128] = jnp.zeros((8, 128), u32)
    st_s[0, 0, 0:8, 0:128] = jnp.zeros((8, 128), f32)
    for k in (0, 1, 2, 3):
        macc_s[k] = jnp.zeros(macc_s.shape[1:], f32)
    w0 = XSPLIT[1]
    cp_x0.wait()
    cp_x1.start()
    macc_s[4] = jnp.zeros(macc_s.shape[1:], f32)
    ln0_s[...] = _pk(ln1(0, w0))
    cp_w1.wait()
    put_h(0, first_use(w1_v, 0, w1t_s, _up(ln0_s[...])))
    cp_wv.wait()
    cp_gw.wait()
    cp_x2.start()
    put_v(0, first_use(wqkv_v, 2 * D, wvt_s, xt_v[:, 0:w0]))
    xp_s[:, 0:w0] = _pk(xt_v[:, 0:w0])
    gw_s[...] = jnp.broadcast_to(gw_v[...].astype(f32).reshape(1, D), (128, D)).T
    cp_x1.wait()
    cp_wqk.start()
    cp_w2.start()
    cp_w3a.start()
    stage_v(256, 256)
    stage_h(256, 256)
    stage_h(512, 512)
    stage_v(512, 512)
    gate_s[...] = gate_of(xt_v[:, 0:TT])
    cp_x2.wait()
    cp_wqk.wait()
    cp_w2.wait()
    cp_w3a.wait()
    cp_wo.start()
    fence()
    cp_w3.start()
    cp_w4.start()
    prep_up(0)
    wqkt_s[...] = _pk(wqkv_v[:, 0:2 * D].T)
    w2t_s[...] = _pk(w2_v[...].T)
    stage_v(1024, 512)
    stage_h(1024, 512)
    stage_h(1536, 512)
    stage_v(1536, 512)
    cp_wo.wait()

    def proj(i, m):
        cols = _span(i * TT, TT)
        xt = _up(xp_s[:, cols])
        zpad = jnp.zeros((HP - DH, TT), f32)

        def heads(y, n):
            return [jnp.concatenate([y[DH * h:DH * (h + 1), :], zpad], axis=0).astype(bf16) for h in range(n)]

        kn = [kh.T for kh in heads(_dot(_up(wqkt_s[D2:D, :]), xt), H)]
        for h in range(H):
            k_s[h, _span(i * T2, T2), :] = _pk(kn[h])
        hw = h_s[:, _span(i * TT, TT + 256)]
        c8 = C4 // 2
        hs = _up(jnp.concatenate([
            hw[0 * c8:1 * c8, 127:127 + TT],
            hw[1 * c8:2 * c8, 129:129 + TT],
            hw[2 * c8:3 * c8, 126:126 + TT],
            hw[3 * c8:4 * c8, 130:130 + TT]], axis=0))

        def qproj(h0, h1):
            y = _dot(_up(wqkt_s[h0 * DH // 2:h1 * DH // 2, :]), xt) * qscale
            for h, qh in enumerate(heads(y, h1 - h0)):
                qt_s[HW * (h + h0):HW * (h + h0 + 1), cols] = _pk(qh)

        qproj(0, 4)
        x1 = xt.astype(f32) + _dot(_up(w2t_s[...]), hs)
        hcols = _span(i * T2, T2)
        macc_s[6, :, hcols] = x1[0:D2, 0:T2]
        b_s[0, :, hcols] = x1[0:D2, T2:TT]
        b_s[1, :, hcols] = x1[D2:D, 0:T2]
        macc_s[5, :, hcols] = x1[D2:D, T2:TT]
        lnf_s[:, cols] = _ln_t(x1)
        s = _dot(kn[0], _up(qt_s[0:HW, 0:TQ]))
        s0_s[cols, :] = s
        m = jnp.maximum(m, jnp.max(s.reshape(TT // 8, 8, TQ), axis=0))
        qproj(4, H)
        wo_f = wo_v[_span(i * GW, GW, 16), :].astype(f32)
        zrows = jnp.zeros((HP - DH, D), f32)
        parts = []
        for j in range(4):
            parts += [wo_f[DH * j:DH * (j + 1), :], zrows]
        wot_s[:, _span(i * 128, 128)] = _pk(jnp.concatenate(parts, axis=0).astype(bf16).T)
        return m

    def proj_body(ii, m):
        for u in range(PU):
            m = proj(ii * PU + u, m)
        return m

    m = lax.fori_loop(0, NT // PU, proj_body, jnp.full((8, TQ), -jnp.inf, f32))
    cp_w3.wait()
    cp_w4.wait()

    sbuf = (s0_s, s1_s, s2_s)

    def ffn_up(tb):
        def prod(k):
            return _dot(_up(w3k_s[k]), _operand(
                _RHS[k], lambda q: lnf_s[(q // 2) * D2:(q // 2 + 1) * D2,
                                         tb * TT + (q % 2) * T2:tb * TT + (q % 2 + 1) * T2]))

        def emit(q, c):
            g_s[q, :, tb * T2:(tb + 1) * T2] = _gelu(c)

        st = st_s.at[tb % 2]
        st[0] = prod(2)
        m5 = prod(4)
        emit(1, st[0] + m5)
        st[2] = m5
        m2 = prod(1)
        st[3] = st[0] - m2
        st[1] = m2
        m4 = prod(3)
        emit(2, st[1] + m4)
        st[2] = m4 - st[2]
        st[0] = prod(0)
        emit(0, st[2] + st[0] + prod(6))
        emit(3, st[3] + st[0] + prod(5))

    def ffn_down(p):
        cols = slice(p * TT, (p + 1) * TT)
        for k in (1, 3, 5, 0, 2, 4, 6):
            macc_s[k, :, cols] += _dot(_up(w4k_s[k]), _operand(_RHS[k], lambda q: g_s[q, :, cols]))

    def body(i, m_in):
        extra = {0: lambda: prep_down(i), 1: lambda: ffn_up(0), 2: lambda: ffn_up(1),
                 3: lambda: ffn_up(2), 4: lambda: ffn_down(0), 5: lambda: ffn_up(3),
                 6: lambda: ffn_down(1), 7: lambda: prep_up(jnp.minimum(i + 1, F // FC - 1))}
        mx = {-1: m_in}
        mrow = {}
        qms = {}
        accs = {}
        for kind, n in _chunk_order():
            u, cc = divmod(n, NC)
            if kind == 0 and cc == LAG and u in extra:
                extra[u]()
            ks = slice(cc * CK, (cc + 1) * CK)
            if kind == 0:
                t1 = i * U + u + 1
                h1 = t1 & (H - 1)
                if cc == 0:
                    qms[u] = _up(qt_s[_span(h1 * HW, HW, HW), _span((t1 >> 4) * TQ, TQ)])
                s = _dot(_up(k_s[h1, cc * CK // 2:(cc + 1) * CK // 2, :]), qms[u])
                sbuf[(u + 1) % NB][ks, :] = s
                mc = jnp.max(s.reshape(CK // 8, 8, TQ), axis=0)
                mx[u] = mc if cc == 0 else jnp.maximum(mx[u], mc)
            else:
                t2 = i * U + u
                hrows = _span((t2 & (H - 1)) * HW, HW, HW)
                if cc == 0:
                    mrow[u] = jnp.max(mx[u - 1], axis=0, keepdims=True)
                p = jnp.exp2(sbuf[u % NB][ks, :] - mrow[u]).astype(bf16)
                pv = _dot(_up(vt_s[hrows, ks]), p)
                accs[u] = pv if cc == 0 else accs[u] + pv
                if cc == NC - 1:
                    acc = accs[u]
                    inv = 1.0 / acc[DH:DH + 1, :]
                    ot_s[hrows, _span((t2 >> 4) * TQ, TQ)] = _pk(acc * inv)
        return mx[U - 1]

    m = lax.fori_loop(0, (NSTEP - 1) // U, body, m)

    s_last = sbuf[(NSTEP - 1) % NB]
    m_last = jnp.max(m, axis=0, keepdims=True)

    def last_pv():
        pacc = None
        for cc in range(NC):
            ks = slice(cc * CK, (cc + 1) * CK)
            p = jnp.exp2(s_last[ks, :] - m_last).astype(bf16)
            pv = _dot(_up(vt_s[(H - 1) * HW:H * HW, ks]), p)
            pacc = pv if pacc is None else pacc + pv
            if cc == NC - 1:
                inv = 1.0 / pacc[DH:DH + 1, :]
                ot_s[(H - 1) * HW:H * HW, S - TQ:S] = _pk(pacc * inv)
            yield

    def mixer_out(q, rows, hc):
        def mk(k):
            return macc_s[k, rows, hc]

        if q == 0:
            return mk(0) + mk(3) - mk(4) + mk(6)
        if q == 1:
            return mk(2) + mk(4) + b_s[0, rows, hc]
        if q == 2:
            return mk(1) + mk(3) + b_s[1, rows, hc]
        return mk(0) - mk(1) + mk(2) + mk(5)

    pvs = last_pv()
    nslots = (NT - 1) * NR - 2
    npv = 0
    RP = D // NR
    for tb in range(NT):
        cols = slice(tb * TT, (tb + 1) * TT)
        hc = slice(tb * T2, (tb + 1) * T2)
        gate = gate_s[...] if tb == 0 else gate_of(_up(xp_s[:, cols]))
        ot = _up(ot_s[:, cols])
        for r in range(NR):
            rows = slice(r * RP, (r + 1) * RP)
            a = _dot(_up(wot_s[r * RP // 2:(r + 1) * RP // 2, :]), ot)
            half, r0 = divmod(r * RP, D2)
            rr = slice(r0, r0 + RP)
            bb = jnp.concatenate([mixer_out(2 * half, rr, hc), mixer_out(2 * half + 1, rr, hc)], axis=1)
            out_v[rows, cols] = (bb + gate * (a - bb)).astype(bf16)
            pltpu.make_async_copy(out_v.at[rows, cols], out_hbm.at[rows, cols], out_sem).start()
            while npv < NC and npv * nslots < (tb * NR + r + 1) * NC:
                next(pvs)
                npv += 1
    pltpu.make_async_copy(out_v, out_hbm, out_sem).wait()


@jax.jit
def pallas_gated_mix__mha_block__mixer_s_mlp__prompt_kernel(
    A_x: jax.Array,
    A_wqkv: jax.Array,
    A_wo: jax.Array,
    B_x: jax.Array,
    B_w1: jax.Array,
    B_w2: jax.Array,
    B_w3: jax.Array,
    B_w4: jax.Array,
    gate_w: jax.Array,
):
    del B_x
    any_spec = pl.BlockSpec(memory_space=pl.ANY)
    out_t = pl.pallas_call(
        _kernel,
        out_shape=jax.ShapeDtypeStruct((D, S), A_x.dtype),
        in_specs=[any_spec] * 8,
        out_specs=any_spec,
        scratch_shapes=[
            pltpu.VMEM((D, S), bf16),
            pltpu.VMEM((D, 3 * D), bf16),
            pltpu.VMEM((D, D), bf16),
            pltpu.VMEM((D, D), bf16),
            pltpu.VMEM((D, D), bf16),
            pltpu.VMEM((D, F), bf16),
            pltpu.VMEM((D, F), bf16),
            pltpu.VMEM((D,), bf16),
            pltpu.VMEM((D, S), bf16),
            pltpu.SemaphoreType.DMA((3,)),
            pltpu.SemaphoreType.DMA(()),
            pltpu.SemaphoreType.REGULAR,
            pltpu.VMEM((D2, D), u32),
            pltpu.VMEM((D2, D), u32),
            pltpu.VMEM((D, D), u32),
            pltpu.VMEM((D2, D), u32),
            pltpu.VMEM((7, F2 // 2, D2), u32),
            pltpu.VMEM((7, D2 // 2, F2), u32),
            pltpu.VMEM((D2, H * HP), u32),
            pltpu.VMEM((D, 128), f32),
            pltpu.VMEM((4, F2, S // 2), f32),
            pltpu.VMEM((7, D2, S // 2), f32),
            pltpu.VMEM((2, 4, F2, T2), f32),
            pltpu.VMEM((D, S), f32),
            pltpu.VMEM((2, D2, S // 2), f32),
            pltpu.VMEM((D2, S), u32),
            pltpu.VMEM((H * HW, S), u32),
            pltpu.VMEM((H, S // 2, HP), u32),
            pltpu.VMEM((H * HW, S), u32),
            pltpu.VMEM((D2, S + 256), u32),
            pltpu.VMEM((S, TQ), f32),
            pltpu.VMEM((S, TQ), f32),
            pltpu.VMEM((S, TQ), f32),
            pltpu.VMEM((H * HW, S), u32),
            pltpu.VMEM((D2, XSPLIT[1]), u32),
            pltpu.VMEM((1, TT), f32),
        ],
        compiler_params=pltpu.CompilerParams(vmem_limit_bytes=100 * 1024 * 1024),
    )(A_x.reshape(S, D).T, A_wqkv, A_wo, B_w1, B_w2, B_w3, B_w4.T, gate_w)
    return out_t.T.reshape(A_x.shape)
```

```python
import math

import jax
import jax.numpy as jnp
from jax import lax
import jax.experimental.pallas as pl
import jax.experimental.pallas.tpu as pltpu

S, D, H, DH, F = 2048, 448, 16, 28, 1792
GW = 4 * DH
HP = 32
HW = HP // 2
TT = 512
TQ = 512
CK = 128
LAG = 2
CATCH = 12
FC = 256
U = 9
PU = 2
NB = 3
NR = 4
C4 = D // 4
D2, F2, T2 = D // 2, FC // 2, TT // 2
NT = S // TT
NSTEP = (S // TQ) * H
NC = S // CK
XSPLIT = (0, 256, 1024, 2048)
KSPLIT = ((0, 256), (256, D))

bf16 = jnp.bfloat16
f32 = jnp.float32
u32 = jnp.uint32

_LHS = ((0, 3, 1), (2, 3, 1), (0, None, 0), (3, None, 0), (0, 1, 1), (2, 0, -1), (1, 3, -1))
_RHS = ((0, 3, 1), (0, None, 0), (1, 3, -1), (2, 0, -1), (3, None, 0), (0, 1, 1), (2, 3, 1))


def _gelu(x):
    c0 = math.sqrt(2.0 / math.pi)
    inner = x * (c0 + (c0 * 0.044715) * (x * x))
    hx = 0.5 * x
    return hx + hx * jnp.tanh(inner)


def _ln_t(x):
    m = jnp.sum(x, axis=0, keepdims=True) * (1.0 / D)
    xc = x - m
    v = jnp.sum(xc * xc, axis=0, keepdims=True) * (1.0 / D)
    return xc * lax.rsqrt(v + 1e-5)


def _pk(x):
    return pltpu.bitcast(x.astype(bf16), u32)


def _up(x):
    return pltpu.bitcast(x, bf16)


def _dot(a, b):
    return jnp.dot(a, b, preferred_element_type=f32)


def _operand(term, quad):
    a, b, sign = term
    if sign == 0:
        return quad(a).astype(bf16)
    ta, tb = quad(a).astype(f32), quad(b).astype(f32)
    return (ta + tb if sign > 0 else ta - tb).astype(bf16)


def _span(c0, w, align=128):
    return slice(c0, c0 + w) if isinstance(c0, int) else pl.ds(pl.multiple_of(c0, align), w)


def _chunk_order():
    ntot = U * NC
    order = []
    done = 0
    for n in range(ntot):
        if n >= ntot - CATCH:
            k = n - (ntot - CATCH) + 1
            target = min(n - LAG + (k * (LAG + 1) + CATCH - 1) // CATCH, ntot)
            while done < target:
                order.append((1, done))
                done += 1
            order.append((0, n))
        else:
            order.append((0, n))
            while done <= n - LAG:
                order.append((1, done))
                done += 1
    assert done == ntot
    return order


def _kernel(xt_hbm, wqkv_hbm, wo_hbm, w1_hbm, w2_hbm, w3_hbm, w4t_hbm, gw_hbm, out_hbm,
            xt_v, wqkv_v, wo_v, w1_v, w2_v, w3_v, w4t_v, gw_v, out_v, sems, out_sem, bar_sem,
            w1t_s, wvt_s, wqkt_s, w2t_s, w3k_s, w4k_s, wot_s, gw_s,
            g_s, macc_s, st_s, lnf_s, b_s,
            xp_s, qt_s, k_s, vt_s, h_s, s0_s, s1_s, s2_s, ot_s, ln0_s, gate_s):
    def cp(src, dst, n):
        return pltpu.make_async_copy(src, dst, sems.at[n])

    def cpx(i, n):
        return cp(xt_hbm.at[:, XSPLIT[i]:XSPLIT[i + 1]], xt_v.at[:, XSPLIT[i]:XSPLIT[i + 1]], n)

    cp_x0 = cpx(0, 0)
    cp_w1 = cp(w1_hbm, w1_v, 1)
    cp_wv = cp(wqkv_hbm.at[:, 2 * D:3 * D], wqkv_v.at[:, 2 * D:3 * D], 2)
    cp_gw = cp(gw_hbm, gw_v, 2)
    cp_x1 = cpx(1, 0)
    cp_x2 = cpx(2, 1)
    cp_wqk = cp(wqkv_hbm.at[:, 0:2 * D], wqkv_v.at[:, 0:2 * D], 1)
    cp_w2 = cp(w2_hbm, w2_v, 1)
    cp_w3a = cp(w3_hbm.at[:, 0:FC], w3_v.at[:, 0:FC], 1)
    cp_wo = cp(wo_hbm, wo_v, 2)
    cp_w3 = cp(w3_hbm.at[:, FC:F], w3_v.at[:, FC:F], 0)
    cp_w4 = cp(w4t_hbm, w4t_v, 0)

    def fence():
        pl.semaphore_signal(bar_sem, 1)
        pl.semaphore_wait(bar_sem, 1)

    cp_x0.start()
    fence()
    cp_w1.start()
    fence()
    cp_wv.start()
    cp_gw.start()

    qscale = (DH ** -0.5) * math.log2(math.e)

    def ln1(c0, w):
        return _ln_t(xt_v[:, c0:c0 + w].astype(f32))

    def put_h(c0, y):
        h_s[:, c0 + 128:c0 + 128 + y.shape[1]] = _pk(_gelu(y))

    def put_v(c0, y):
        w = y.shape[1]
        rid = lax.broadcasted_iota(jnp.int32, (HP - DH, w), 0)
        tail = jnp.where(rid == 0, 1.0, 0.0).astype(f32)
        for h in range(H):
            vt_s[HW * h:HW * (h + 1), c0:c0 + w] = _pk(
                jnp.concatenate([y[DH * h:DH * (h + 1), :], tail], axis=0))

    def first_use(w_ref, c0, wt_ref, rhs):
        y = None
        for k0, k1 in KSPLIT:
            wt = w_ref[k0:k1, c0:c0 + D].T
            wt_ref[:, k0:k1] = _pk(wt)
            part = _dot(wt, rhs[k0:k1, :])
            y = part if y is None else y + part
        return y

    def prep_up(c):
        for k in range(7):
            w3k_s[k] = _pk(_operand(_LHS[k], lambda q: w3_v[(q % 2) * D2:(q % 2 + 1) * D2,
                                                            _span(c * FC + (q // 2) * F2, F2)]).T)

    def prep_down(c):
        for k in range(7):
            w4k_s[k] = _pk(_operand(_LHS[k], lambda q: w4t_v[(q // 2) * D2:(q // 2 + 1) * D2,
                                                             _span(c * FC + (q % 2) * F2, F2)]))

    def stage_v(c0, w):
        xt = xt_v[:, c0:c0 + w]
        xp_s[:, c0:c0 + w] = _pk(xt)
        put_v(c0, _dot(_up(wvt_s[...]), xt))

    def stage_h(c0, w):
        put_h(c0, _dot(_up(w1t_s[...]), ln1(c0, w).astype(bf16)))

    def gate_of(x):
        gwc = gw_s[...]
        z = jnp.sum(x.astype(f32) * jnp.concatenate([gwc] * (TT // 128), axis=1), axis=0, keepdims=True)
        return 1.0 / (1.0 + jnp.exp(-z))

    h_s[:, 0:128] = jnp.zeros((D2, 128), u32)
    h_s[:, S + 128:S + 256] = jnp.zeros((D2, 128), u32)
    for sb in (s1_s, s2_s):
        sb[0:8, :] = jnp.zeros((8, TQ), f32)
    g_s[0, 0:8, 0:128] = jnp.zeros((8, 128), f32)
    w4k_s[0, 0:8, 0:128] = jnp.zeros((8, 128), u32)
    st_s[0, 0, 0:8, 0:128] = jnp.zeros((8, 128), f32)
    for k in (0, 1, 2, 3):
        macc_s[k] = jnp.zeros(macc_s.shape[1:], f32)
    w0 = XSPLIT[1]
    cp_x0.wait()
    cp_x1.start()
    macc_s[4] = jnp.zeros(macc_s.shape[1:], f32)
    ln0_s[...] = _pk(ln1(0, w0))
    cp_w1.wait()
    put_h(0, first_use(w1_v, 0, w1t_s, _up(ln0_s[...])))
    cp_wv.wait()
    cp_gw.wait()
    cp_x2.start()
    put_v(0, first_use(wqkv_v, 2 * D, wvt_s, xt_v[:, 0:w0]))
    xp_s[:, 0:w0] = _pk(xt_v[:, 0:w0])
    gw_s[...] = jnp.broadcast_to(gw_v[...].astype(f32).reshape(1, D), (128, D)).T
    cp_x1.wait()
    cp_wqk.start()
    cp_w2.start()
    cp_w3a.start()
    stage_v(256, 256)
    stage_h(256, 256)
    stage_h(512, 512)
    stage_v(512, 512)
    gate_s[...] = gate_of(xt_v[:, 0:TT])
    cp_x2.wait()
    cp_wqk.wait()
    cp_w2.wait()
    cp_w3a.wait()
    cp_wo.start()
    fence()
    cp_w3.start()
    cp_w4.start()
    prep_up(0)
    wqkt_s[...] = _pk(wqkv_v[:, 0:2 * D].T)
    w2t_s[...] = _pk(w2_v[...].T)
    stage_v(1024, 512)
    stage_h(1024, 512)
    stage_h(1536, 512)
    stage_v(1536, 512)
    cp_wo.wait()

    def proj(i, odd, m):
        cols = _span(i * TT, TT)
        xt = _up(xp_s[:, cols])
        zpad = jnp.zeros((HP - DH, TT), f32)

        def heads(y, n):
            return [jnp.concatenate([y[DH * h:DH * (h + 1), :], zpad], axis=0).astype(bf16) for h in range(n)]

        kn = [kh.T for kh in heads(_dot(_up(wqkt_s[D2:D, :]), xt), H)]
        for h in range(H):
            k_s[h, _span(i * T2, T2), :] = _pk(kn[h])
        hw = h_s[:, _span(i * TT, TT + 256)]
        c8 = C4 // 2
        hs = _up(jnp.concatenate([
            hw[0 * c8:1 * c8, 127:127 + TT],
            hw[1 * c8:2 * c8, 129:129 + TT],
            hw[2 * c8:3 * c8, 126:126 + TT],
            hw[3 * c8:4 * c8, 130:130 + TT]], axis=0))

        def qproj(h0, h1):
            y = _dot(_up(wqkt_s[h0 * DH // 2:h1 * DH // 2, :]), xt) * qscale
            for h, qh in enumerate(heads(y, h1 - h0)):
                qt_s[HW * (h + h0):HW * (h + h0 + 1), cols] = _pk(qh)

        qproj(0, 4)
        x1 = xt.astype(f32) + _dot(_up(w2t_s[...]), hs)
        hcols = _span((i - odd) * T2, TT)
        if odd:
            b_s[0, :, hcols] = x1[0:D2, :]
            macc_s[5, :, hcols] = x1[D2:D, :]
        else:
            macc_s[6, :, hcols] = x1[0:D2, :]
            b_s[1, :, hcols] = x1[D2:D, :]
        lnf_s[:, cols] = _ln_t(x1)
        s = _dot(kn[0], _up(qt_s[0:HW, 0:TQ]))
        s0_s[cols, :] = s
        m = jnp.maximum(m, jnp.max(s.reshape(TT // 8, 8, TQ), axis=0))
        qproj(4, H)
        wo_f = wo_v[_span(i * GW, GW, 16), :].astype(f32)
        zrows = jnp.zeros((HP - DH, D), f32)
        parts = []
        for j in range(4):
            parts += [wo_f[DH * j:DH * (j + 1), :], zrows]
        wot_s[:, _span(i * 128, 128)] = _pk(jnp.concatenate(parts, axis=0).astype(bf16).T)
        return m

    def proj_body(ii, m):
        for u in range(PU):
            m = proj(ii * PU + u, u % 2, m)
        return m

    m = lax.fori_loop(0, NT // PU, proj_body, jnp.full((8, TQ), -jnp.inf, f32))
    cp_w3.wait()
    cp_w4.wait()

    sbuf = (s0_s, s1_s, s2_s)

    def ffn_up(p):
        def prod(k):
            return _dot(_up(w3k_s[k]), _operand(
                _RHS[k], lambda q: lnf_s[(q // 2) * D2:(q // 2 + 1) * D2,
                                         (2 * p + q % 2) * TT:(2 * p + q % 2 + 1) * TT]))

        def emit(q, c):
            g_s[q, :, p * TT:(p + 1) * TT] = _gelu(c)

        st = st_s.at[p]
        st[0] = prod(4)
        m3 = prod(2)
        emit(1, st[0] + m3)
        st[3] = m3
        st[1] = prod(1)
        m4 = prod(3)
        emit(2, st[1] + m4)
        st[2] = m4 - st[0]
        st[2] += prod(6)
        m1 = prod(0)
        emit(0, st[2] + m1)
        st[3] = st[3] - st[1] + m1
        emit(3, st[3] + prod(5))

    def ffn_down(p):
        cols = slice(p * TT, (p + 1) * TT)
        for k in (1, 3, 5, 0, 2, 4, 6):
            macc_s[k, :, cols] += _dot(_up(w4k_s[k]), _operand(_RHS[k], lambda q: g_s[q, :, cols]))

    def body(i, m_in):
        extra = {0: lambda: prep_down(i), 1: lambda: ffn_up(0), 2: lambda: ffn_up(1),
                 3: lambda: ffn_down(0), 4: lambda: ffn_down(1),
                 5: lambda: prep_up(jnp.minimum(i + 1, F // FC - 1))}
        mx = {-1: m_in}
        mrow = {}
        qms = {}
        accs = {}
        for kind, n in _chunk_order():
            u, cc = divmod(n, NC)
            if kind == 0 and cc == LAG and u in extra:
                extra[u]()
            ks = slice(cc * CK, (cc + 1) * CK)
            if kind == 0:
                t1 = i * U + u + 1
                h1 = t1 & (H - 1)
                if cc == 0:
                    qms[u] = _up(qt_s[_span(h1 * HW, HW, HW), _span((t1 >> 4) * TQ, TQ)])
                s = _dot(_up(k_s[h1, cc * CK // 2:(cc + 1) * CK // 2, :]), qms[u])
                sbuf[(u + 1) % NB][ks, :] = s
                mc = jnp.max(s.reshape(CK // 8, 8, TQ), axis=0)
                mx[u] = mc if cc == 0 else jnp.maximum(mx[u], mc)
            else:
                t2 = i * U + u
                hrows = _span((t2 & (H - 1)) * HW, HW, HW)
                if cc == 0:
                    mrow[u] = jnp.max(mx[u - 1], axis=0, keepdims=True)
                p = jnp.exp2(sbuf[u % NB][ks, :] - mrow[u]).astype(bf16)
                pv = _dot(_up(vt_s[hrows, ks]), p)
                accs[u] = pv if cc == 0 else accs[u] + pv
                if cc == NC - 1:
                    acc = accs[u]
                    inv = 1.0 / acc[DH:DH + 1, :]
                    ot_s[hrows, _span((t2 >> 4) * TQ, TQ)] = _pk(acc * inv)
        return mx[U - 1]

    m = lax.fori_loop(0, (NSTEP - 1) // U, body, m)

    s_last = sbuf[(NSTEP - 1) % NB]
    m_last = jnp.max(m, axis=0, keepdims=True)

    def last_pv():
        pacc = None
        for cc in range(NC):
            ks = slice(cc * CK, (cc + 1) * CK)
            p = jnp.exp2(s_last[ks, :] - m_last).astype(bf16)
            pv = _dot(_up(vt_s[(H - 1) * HW:H * HW, ks]), p)
            pacc = pv if pacc is None else pacc + pv
            if cc == NC - 1:
                inv = 1.0 / pacc[DH:DH + 1, :]
                ot_s[(H - 1) * HW:H * HW, S - TQ:S] = _pk(pacc * inv)
            yield

    def mixer_out(q, rows, hc):
        def mk(k):
            return macc_s[k, rows, hc]

        if q == 0:
            return mk(0) + mk(3) - mk(4) + mk(6)
        if q == 1:
            return mk(2) + mk(4) + b_s[0, rows, hc]
        if q == 2:
            return mk(1) + mk(3) + b_s[1, rows, hc]
        return mk(0) - mk(1) + mk(2) + mk(5)

    pvs = last_pv()
    nslots = (NT - 1) * NR - 2
    npv = 0
    RP = D // NR
    for tb in range(NT):
        cols = slice(tb * TT, (tb + 1) * TT)
        hc = slice((tb // 2) * TT, (tb // 2 + 1) * TT)
        gate = gate_s[...] if tb == 0 else gate_of(_up(xp_s[:, cols]))
        ot = _up(ot_s[:, cols])
        for r in range(NR):
            rows = slice(r * RP, (r + 1) * RP)
            a = _dot(_up(wot_s[r * RP // 2:(r + 1) * RP // 2, :]), ot)
            half, r0 = divmod(r * RP, D2)
            bb = mixer_out(2 * half + tb % 2, slice(r0, r0 + RP), hc)
            out_v[rows, cols] = (bb + gate * (a - bb)).astype(bf16)
            pltpu.make_async_copy(out_v.at[rows, cols], out_hbm.at[rows, cols], out_sem).start()
            while npv < NC and npv * nslots < (tb * NR + r + 1) * NC:
                next(pvs)
                npv += 1
    pltpu.make_async_copy(out_v, out_hbm, out_sem).wait()


@jax.jit
def pallas_gated_mix__mha_block__mixer_s_mlp__prompt_kernel(
    A_x: jax.Array,
    A_wqkv: jax.Array,
    A_wo: jax.Array,
    B_x: jax.Array,
    B_w1: jax.Array,
    B_w2: jax.Array,
    B_w3: jax.Array,
    B_w4: jax.Array,
    gate_w: jax.Array,
):
    del B_x
    any_spec = pl.BlockSpec(memory_space=pl.ANY)
    out_t = pl.pallas_call(
        _kernel,
        out_shape=jax.ShapeDtypeStruct((D, S), A_x.dtype),
        in_specs=[any_spec] * 8,
        out_specs=any_spec,
        scratch_shapes=[
            pltpu.VMEM((D, S), bf16),
            pltpu.VMEM((D, 3 * D), bf16),
            pltpu.VMEM((D, D), bf16),
            pltpu.VMEM((D, D), bf16),
            pltpu.VMEM((D, D), bf16),
            pltpu.VMEM((D, F), bf16),
            pltpu.VMEM((D, F), bf16),
            pltpu.VMEM((D,), bf16),
            pltpu.VMEM((D, S), bf16),
            pltpu.SemaphoreType.DMA((3,)),
            pltpu.SemaphoreType.DMA(()),
            pltpu.SemaphoreType.REGULAR,
            pltpu.VMEM((D2, D), u32),
            pltpu.VMEM((D2, D), u32),
            pltpu.VMEM((D, D), u32),
            pltpu.VMEM((D2, D), u32),
            pltpu.VMEM((7, F2 // 2, D2), u32),
            pltpu.VMEM((7, D2 // 2, F2), u32),
            pltpu.VMEM((D2, H * HP), u32),
            pltpu.VMEM((D, 128), f32),
            pltpu.VMEM((4, F2, S // 2), f32),
            pltpu.VMEM((7, D2, S // 2), f32),
            pltpu.VMEM((2, 4, F2, TT), f32),
            pltpu.VMEM((D, S), f32),
            pltpu.VMEM((2, D2, S // 2), f32),
            pltpu.VMEM((D2, S), u32),
            pltpu.VMEM((H * HW, S), u32),
            pltpu.VMEM((H, S // 2, HP), u32),
            pltpu.VMEM((H * HW, S), u32),
            pltpu.VMEM((D2, S + 256), u32),
            pltpu.VMEM((S, TQ), f32),
            pltpu.VMEM((S, TQ), f32),
            pltpu.VMEM((S, TQ), f32),
            pltpu.VMEM((H * HW, S), u32),
            pltpu.VMEM((D2, XSPLIT[1]), u32),
            pltpu.VMEM((1, TT), f32),
        ],
        compiler_params=pltpu.CompilerParams(vmem_limit_bytes=100 * 1024 * 1024),
    )(A_x.reshape(S, D).T, A_wqkv, A_wo, B_w1, B_w2, B_w3, B_w4.T, gate_w)
    return out_t.T.reshape(A_x.shape)
```

```python
import math

import jax
import jax.numpy as jnp
from jax import lax
import jax.experimental.pallas as pl
import jax.experimental.pallas.tpu as pltpu

S, D, H, DH, F = 2048, 448, 16, 28, 1792
GW = 4 * DH
HP = 32
HW = HP // 2
TT = 512
TQ = 512
CK = 128
LAG = 2
CATCH = 12
FC = 256
U = 9
PU = 2
NB = 3
C4 = D // 4
D2, F2, T2 = D // 2, FC // 2, TT // 2
NT = S // TT
NSTEP = (S // TQ) * H
NC = S // CK
XSPLIT = (0, 256, 1024, 2048)
KSPLIT = ((0, 256), (256, D))

bf16 = jnp.bfloat16
f32 = jnp.float32
u32 = jnp.uint32

_LHS = ((0, 3, 1), (2, 3, 1), (0, None, 0), (3, None, 0), (0, 1, 1), (2, 0, -1), (1, 3, -1))
_RHS = ((0, 3, 1), (0, None, 0), (1, 3, -1), (2, 0, -1), (3, None, 0), (0, 1, 1), (2, 3, 1))


def _gelu(x, half=0.5):
    c0 = math.sqrt(2.0 / math.pi)
    inner = x * (c0 + (c0 * 0.044715) * (x * x))
    hx = half * x
    return hx + hx * jnp.tanh(inner)


def _ln_t(x):
    m = jnp.sum(x, axis=0, keepdims=True) * (1.0 / D)
    xc = x - m
    v = jnp.sum(xc * xc, axis=0, keepdims=True) * (1.0 / D)
    return xc * lax.rsqrt(v + 1e-5)


def _pk(x):
    return pltpu.bitcast(x.astype(bf16), u32)


def _up(x):
    return pltpu.bitcast(x, bf16)


def _dot(a, b):
    return jnp.dot(a, b, preferred_element_type=f32)


def _operand(term, quad):
    a, b, sign = term
    if sign == 0:
        return quad(a).astype(bf16)
    ta, tb = quad(a).astype(f32), quad(b).astype(f32)
    return (ta + tb if sign > 0 else ta - tb).astype(bf16)


def _strassen(prod, st, emit):
    st[0] = prod(4)
    m3 = prod(2)
    emit(1, st[0] + m3)
    st[3] = m3
    st[1] = prod(1)
    m4 = prod(3)
    emit(2, st[1] + m4)
    st[2] = m4 - st[0]
    st[2] += prod(6)
    m1 = prod(0)
    emit(0, st[2] + m1)
    st[3] = st[3] - st[1] + m1
    emit(3, st[3] + prod(5))


def _span(c0, w, align=128):
    return slice(c0, c0 + w) if isinstance(c0, int) else pl.ds(pl.multiple_of(c0, align), w)


def _chunk_order():
    ntot = U * NC
    order = []
    done = 0
    for n in range(ntot):
        if n >= ntot - CATCH:
            k = n - (ntot - CATCH) + 1
            target = min(n - LAG + (k * (LAG + 1) + CATCH - 1) // CATCH, ntot)
            while done < target:
                order.append((1, done))
                done += 1
            order.append((0, n))
        else:
            order.append((0, n))
            while done <= n - LAG:
                order.append((1, done))
                done += 1
    assert done == ntot
    return order


def _kernel(xt_hbm, wqkv_hbm, wo_hbm, w1_hbm, w2_hbm, w3_hbm, w4t_hbm, gw_hbm, out_hbm,
            xt_v, wqkv_v, wo_v, w1_v, w2_v, w3_v, w4t_v, gw_v, out_v, sems, out_sem, bar_sem,
            w1t_s, wvt_s, wqkt_s, w2t_s, w3k_s, w4k_s, wot_s, gw_s,
            g_s, macc_s, st_s, lnf_s, b_s,
            xp_s, qt_s, k_s, vt_s, h_s, s0_s, s1_s, s2_s, ot_s, ln0_s, gate_s, wok_s, sto_s, wvk_s):
    def cp(src, dst, n):
        return pltpu.make_async_copy(src, dst, sems.at[n])

    def cpx(i, n):
        return cp(xt_hbm.at[:, XSPLIT[i]:XSPLIT[i + 1]], xt_v.at[:, XSPLIT[i]:XSPLIT[i + 1]], n)

    cp_x0 = cpx(0, 0)
    cp_w1 = cp(w1_hbm, w1_v, 1)
    cp_wv = cp(wqkv_hbm.at[:, 2 * D:3 * D], wqkv_v.at[:, 2 * D:3 * D], 2)
    cp_gw = cp(gw_hbm, gw_v, 2)
    cp_x1 = cpx(1, 0)
    cp_x2 = cpx(2, 1)
    cp_wqk = cp(wqkv_hbm.at[:, 0:2 * D], wqkv_v.at[:, 0:2 * D], 1)
    cp_w2 = cp(w2_hbm, w2_v, 1)
    cp_w3a = cp(w3_hbm.at[:, 0:FC], w3_v.at[:, 0:FC], 1)
    cp_wo = cp(wo_hbm, wo_v, 2)
    cp_w3 = cp(w3_hbm.at[:, FC:F], w3_v.at[:, FC:F], 0)
    cp_w4 = cp(w4t_hbm, w4t_v, 0)

    def fence():
        pl.semaphore_signal(bar_sem, 1)
        pl.semaphore_wait(bar_sem, 1)

    cp_x0.start()
    fence()
    cp_w1.start()
    fence()
    cp_wv.start()
    cp_gw.start()

    qscale = (DH ** -0.5) * math.log2(math.e)

    def ln1(c0, w):
        return _ln_t(xt_v[:, c0:c0 + w].astype(f32))

    def put_h(c0, y):
        h_s[:, c0 + 128:c0 + 128 + y.shape[1]] = _pk(_gelu(y))

    def put_v(c0, y, h0=0):
        w = y.shape[1]
        rid = lax.broadcasted_iota(jnp.int32, (HP - DH, w), 0)
        tail = jnp.where(rid == 0, 1.0, 0.0).astype(f32)
        for h in range(y.shape[0] // DH):
            vt_s[HW * (h0 + h):HW * (h0 + h + 1), c0:c0 + w] = _pk(
                jnp.concatenate([y[DH * h:DH * (h + 1), :], tail], axis=0))

    def first_use(w_ref, c0, wt_ref, rhs):
        y = None
        for k0, k1 in KSPLIT:
            wt = w_ref[k0:k1, c0:c0 + D].T
            wt_ref[:, k0:k1] = _pk(wt)
            part = _dot(wt, rhs[k0:k1, :])
            y = part if y is None else y + part
        return y

    def prep_up(c):
        for k in range(7):
            w3k_s[k] = _pk(_operand(_LHS[k], lambda q: w3_v[(q % 2) * D2:(q % 2 + 1) * D2,
                                                            _span(c * FC + (q // 2) * F2, F2)]).T)

    def prep_down(c):
        for k in range(7):
            w4k_s[k] = _pk(_operand(_LHS[k], lambda q: w4t_v[(q // 2) * D2:(q // 2 + 1) * D2,
                                                             _span(c * FC + (q % 2) * F2, F2)]))

    def stage_v(c0, w, slot=0):
        xp_s[:, c0:c0 + w] = _pk(xt_v[:, c0:c0 + w])
        if w < TT:
            put_v(c0, _dot(_up(wvt_s[0]), xt_v[0:D2, c0:c0 + w]) + _dot(_up(wvt_s[1]), xt_v[D2:D, c0:c0 + w]))
            return

        def prod(k):
            return _dot(_up(wvk_s[k]), _operand(
                _RHS[k], lambda q: xt_v[(q // 2) * D2:(q // 2 + 1) * D2,
                                        c0 + (q % 2) * T2:c0 + (q % 2 + 1) * T2]))

        _strassen(prod, sto_s.at[slot], lambda q, c: put_v(c0 + (q % 2) * T2, c, (q // 2) * (H // 2)))

    def stage_h(c0, w):
        xf = xt_v[:, c0:c0 + w].astype(f32)
        gate_s[:, c0:c0 + w] = gate_of(xf)
        put_h(c0, _dot(_up(w1t_s[...]), _ln_t(xf).astype(bf16)))

    def gate_of(x):
        gwc = gw_s[...]
        z = jnp.sum(x.astype(f32) * jnp.concatenate([gwc] * (x.shape[1] // 128), axis=1), axis=0, keepdims=True)
        return 1.0 / (1.0 + jnp.exp(-z))

    h_s[:, 0:128] = jnp.zeros((D2, 128), u32)
    h_s[:, S + 128:S + 256] = jnp.zeros((D2, 128), u32)
    for sb in (s1_s, s2_s):
        sb[0:8, :] = jnp.zeros((8, TQ), f32)
    g_s[0, 0:8, 0:128] = jnp.zeros((8, 128), f32)
    w4k_s[0, 0:8, 0:128] = jnp.zeros((8, 128), u32)
    st_s[0, 0, 0:8, 0:128] = jnp.zeros((8, 128), f32)
    sto_s[0, 0, 0:8, 0:128] = jnp.zeros((8, 128), f32)
    wok_s[0, 0:8, 0:128] = jnp.zeros((8, 128), u32)
    for k in (0, 1, 2, 3):
        macc_s[k] = jnp.zeros(macc_s.shape[1:], f32)
    w0 = XSPLIT[1]
    cp_x0.wait()
    cp_x1.start()
    macc_s[4] = jnp.zeros(macc_s.shape[1:], f32)
    ln0_s[...] = _pk(ln1(0, w0))
    cp_w1.wait()
    put_h(0, first_use(w1_v, 0, w1t_s, _up(ln0_s[...])))
    cp_wv.wait()
    cp_gw.wait()
    cp_x2.start()
    wv_t = [wqkv_v[j * D2:(j + 1) * D2, 2 * D:3 * D].T for j in range(2)]
    for j in range(2):
        wvt_s[j] = _pk(wv_t[j])
    put_v(0, _dot(wv_t[0], xt_v[0:D2, 0:w0]) + _dot(wv_t[1], xt_v[D2:D, 0:w0]))
    xp_s[:, 0:w0] = _pk(xt_v[:, 0:w0])
    gw_s[...] = jnp.broadcast_to(gw_v[...].astype(f32).reshape(1, D), (128, D)).T
    cp_x1.wait()
    cp_wqk.start()
    cp_w2.start()
    cp_w3a.start()
    for k in (4, 2, 1, 3, 6, 0, 5):
        wvk_s[k] = _pk(_operand(
            _LHS[k], lambda q: _up(wvt_s[q % 2, (q // 2) * D2 // 2:(q // 2 + 1) * D2 // 2, :])))
    stage_v(256, 256)
    stage_h(256, 256)
    stage_h(512, 512)
    stage_v(512, 512)
    gate_s[:, 0:w0] = gate_of(xt_v[:, 0:w0])
    cp_x2.wait()
    cp_wqk.wait()
    cp_w2.wait()
    cp_w3a.wait()
    cp_wo.start()
    fence()
    cp_w3.start()
    cp_w4.start()
    prep_up(0)
    wqkt_s[...] = _pk(wqkv_v[:, 0:2 * D].T)
    w2t_s[...] = _pk(w2_v[...].T)
    stage_v(1024, 512)
    stage_h(1024, 512)
    stage_h(1536, 512)
    stage_v(1536, 512, 1)
    cp_wo.wait()

    def proj(i, odd, m):
        cols = _span(i * TT, TT)
        xt = _up(xp_s[:, cols])
        zpad = jnp.zeros((HP - DH, TT), f32)

        def heads(y, n):
            return [jnp.concatenate([y[DH * h:DH * (h + 1), :], zpad], axis=0).astype(bf16) for h in range(n)]

        kn = [kh.T for kh in heads(_dot(_up(wqkt_s[D2:D, :]), xt), H)]
        for h in range(H):
            k_s[h, _span(i * T2, T2), :] = _pk(kn[h])
        hw = h_s[:, _span(i * TT, TT + 256)]
        c8 = C4 // 2
        hs = _up(jnp.concatenate([
            hw[0 * c8:1 * c8, 127:127 + TT],
            hw[1 * c8:2 * c8, 129:129 + TT],
            hw[2 * c8:3 * c8, 126:126 + TT],
            hw[3 * c8:4 * c8, 130:130 + TT]], axis=0))

        def qproj(h0, h1):
            y = _dot(_up(wqkt_s[h0 * DH // 2:h1 * DH // 2, :]), xt) * qscale
            for h, qh in enumerate(heads(y, h1 - h0)):
                qt_s[HW * (h + h0):HW * (h + h0 + 1), cols] = _pk(qh)

        qproj(0, 4)
        x1 = xt.astype(f32) + _dot(_up(w2t_s[...]), hs)
        hcols = _span((i - odd) * T2, TT)
        xs = x1 * (1.0 - gate_s[:, cols])
        if odd:
            b_s[0, :, hcols] = xs[0:D2, :]
            macc_s[5, :, hcols] = xs[D2:D, :]
        else:
            macc_s[6, :, hcols] = xs[0:D2, :]
            b_s[1, :, hcols] = xs[D2:D, :]
        lnf_s[:, cols] = _ln_t(x1)
        s = _dot(kn[0], _up(qt_s[0:HW, 0:TQ]))
        s0_s[cols, :] = s
        m = jnp.maximum(m, jnp.max(s.reshape(TT // 8, 8, TQ), axis=0))
        qproj(4, H)
        wo_f = wo_v[_span(i * GW, GW, 16), :].astype(f32)
        zrows = jnp.zeros((HP - DH, D), f32)
        parts = []
        for j in range(4):
            parts += [wo_f[DH * j:DH * (j + 1), :], zrows]
        wot_s[:, _span(i * 128, 128)] = _pk(jnp.concatenate(parts, axis=0).astype(bf16).T)
        return m

    def proj_body(ii, m):
        for u in range(PU):
            m = proj(ii * PU + u, u % 2, m)
        return m

    m = lax.fori_loop(0, NT // PU, proj_body, jnp.full((8, TQ), -jnp.inf, f32))
    cp_w3.wait()
    cp_w4.wait()

    sbuf = (s0_s, s1_s, s2_s)

    def ffn_up(p):
        def prod(k):
            return _dot(_up(w3k_s[k]), _operand(
                _RHS[k], lambda q: lnf_s[(q // 2) * D2:(q // 2 + 1) * D2,
                                         (2 * p + q % 2) * TT:(2 * p + q % 2 + 1) * TT]))

        def emit(q, c):
            tb = 2 * p + q % 2
            g_s[q, :, p * TT:(p + 1) * TT] = _gelu(c, 0.5 - 0.5 * gate_s[:, tb * TT:(tb + 1) * TT])

        _strassen(prod, st_s.at[p], emit)

    def ffn_down(p):
        cols = slice(p * TT, (p + 1) * TT)
        for k in (1, 3, 5, 0, 2, 4, 6):
            macc_s[k, :, cols] += _dot(_up(w4k_s[k]), _operand(_RHS[k], lambda q: g_s[q, :, cols]))

    def body(i, m_in):
        extra = {0: lambda: prep_down(i), 1: lambda: ffn_up(0), 2: lambda: ffn_up(1),
                 3: lambda: ffn_down(0), 4: lambda: ffn_down(1),
                 5: lambda: prep_up(jnp.minimum(i + 1, F // FC - 1))}
        mx = {-1: m_in}
        mrow = {}
        qms = {}
        accs = {}
        for kind, n in _chunk_order():
            u, cc = divmod(n, NC)
            if kind == 0 and cc == LAG and u in extra:
                extra[u]()
            ks = slice(cc * CK, (cc + 1) * CK)
            if kind == 0:
                t1 = i * U + u + 1
                h1 = t1 & (H - 1)
                if cc == 0:
                    qms[u] = _up(qt_s[_span(h1 * HW, HW, HW), _span((t1 >> 4) * TQ, TQ)])
                s = _dot(_up(k_s[h1, cc * CK // 2:(cc + 1) * CK // 2, :]), qms[u])
                sbuf[(u + 1) % NB][ks, :] = s
                mc = jnp.max(s.reshape(CK // 8, 8, TQ), axis=0)
                mx[u] = mc if cc == 0 else jnp.maximum(mx[u], mc)
            else:
                t2 = i * U + u
                hrows = _span((t2 & (H - 1)) * HW, HW, HW)
                if cc == 0:
                    mrow[u] = jnp.max(mx[u - 1], axis=0, keepdims=True)
                p = jnp.exp2(sbuf[u % NB][ks, :] - mrow[u]).astype(bf16)
                pv = _dot(_up(vt_s[hrows, ks]), p)
                accs[u] = pv if cc == 0 else accs[u] + pv
                if cc == NC - 1:
                    acc = accs[u]
                    qcols = _span((t2 >> 4) * TQ, TQ)
                    inv = gate_s[:, qcols] / acc[DH:DH + 1, :]
                    ot_s[_span((t2 & (H - 1)) * HP, HP, HP), qcols] = acc * inv
        return mx[U - 1]

    m = lax.fori_loop(0, (NSTEP - 1) // U, body, m)

    s_last = sbuf[(NSTEP - 1) % NB]
    m_last = jnp.max(m, axis=0, keepdims=True)

    def last_pv():
        pacc = None
        for cc in range(NC):
            ks = slice(cc * CK, (cc + 1) * CK)
            p = jnp.exp2(s_last[ks, :] - m_last).astype(bf16)
            pv = _dot(_up(vt_s[(H - 1) * HW:H * HW, ks]), p)
            pacc = pv if pacc is None else pacc + pv
            if cc == NC - 1:
                inv = gate_s[:, S - TQ:S] / pacc[DH:DH + 1, :]
                ot_s[(H - 1) * HP:H * HP, S - TQ:S] = pacc * inv
            yield

    pvs = last_pv()
    KH = H * HP // 2
    for k in (4, 2, 1, 3, 6, 0, 5):
        wok_s[k] = _pk(_operand(
            _LHS[k], lambda q: _up(wot_s[(q // 2) * D2 // 2:(q // 2 + 1) * D2 // 2,
                                         (q % 2) * KH:(q % 2 + 1) * KH])))
    nprod = [0]

    def out_pair(p, j):
        hc = slice(p * TT + j * T2, p * TT + (j + 1) * T2)

        def tcols(q):
            c0 = (2 * p + q % 2) * TT + j * T2
            return slice(c0, c0 + T2)

        def prod(k):
            rhs = _operand(_RHS[k], lambda q: ot_s[(q // 2) * KH:(q // 2 + 1) * KH, tcols(q)])
            cuts = (0, 40, 72, D2 // 2) if nprod[0] < NC // 2 else (0, D2 // 2)
            nprod[0] += 1
            parts = []
            for a, b in zip(cuts[:-1], cuts[1:]):
                if a:
                    next(pvs)
                parts.append(_dot(_up(wok_s[k, a:b, :]), rhs))
            return macc_s[k, :, hc] + jnp.concatenate(parts, axis=0)

        def emit(q, c):
            rows = slice((q // 2) * D2, (q // 2 + 1) * D2)
            if q in (1, 2):
                c = c + b_s[q - 1, :, hc]
            out_v[rows, tcols(q)] = c.astype(bf16)
            pltpu.make_async_copy(out_v.at[rows, tcols(q)], out_hbm.at[rows, tcols(q)], out_sem).start()

        _strassen(prod, sto_s.at[j], emit)

    for p in range(2):
        for j in range(2):
            out_pair(p, j)
    pltpu.make_async_copy(out_v, out_hbm, out_sem).wait()


@jax.jit
def pallas_gated_mix__mha_block__mixer_s_mlp__prompt_kernel(
    A_x: jax.Array,
    A_wqkv: jax.Array,
    A_wo: jax.Array,
    B_x: jax.Array,
    B_w1: jax.Array,
    B_w2: jax.Array,
    B_w3: jax.Array,
    B_w4: jax.Array,
    gate_w: jax.Array,
):
    del B_x
    any_spec = pl.BlockSpec(memory_space=pl.ANY)
    out_t = pl.pallas_call(
        _kernel,
        out_shape=jax.ShapeDtypeStruct((D, S), A_x.dtype),
        in_specs=[any_spec] * 8,
        out_specs=any_spec,
        scratch_shapes=[
            pltpu.VMEM((D, S), bf16),
            pltpu.VMEM((D, 3 * D), bf16),
            pltpu.VMEM((D, D), bf16),
            pltpu.VMEM((D, D), bf16),
            pltpu.VMEM((D, D), bf16),
            pltpu.VMEM((D, F), bf16),
            pltpu.VMEM((D, F), bf16),
            pltpu.VMEM((D,), bf16),
            pltpu.VMEM((D, S), bf16),
            pltpu.SemaphoreType.DMA((3,)),
            pltpu.SemaphoreType.DMA(()),
            pltpu.SemaphoreType.REGULAR,
            pltpu.VMEM((D2, D), u32),
            pltpu.VMEM((2, D2, D2), u32),
            pltpu.VMEM((D, D), u32),
            pltpu.VMEM((D2, D), u32),
            pltpu.VMEM((7, F2 // 2, D2), u32),
            pltpu.VMEM((7, D2 // 2, F2), u32),
            pltpu.VMEM((D2, H * HP), u32),
            pltpu.VMEM((D, 128), f32),
            pltpu.VMEM((4, F2, S // 2), f32),
            pltpu.VMEM((7, D2, S // 2), f32),
            pltpu.VMEM((2, 4, F2, TT), f32),
            pltpu.VMEM((D, S), f32),
            pltpu.VMEM((2, D2, S // 2), f32),
            pltpu.VMEM((D2, S), u32),
            pltpu.VMEM((H * HW, S), u32),
            pltpu.VMEM((H, S // 2, HP), u32),
            pltpu.VMEM((H * HW, S), u32),
            pltpu.VMEM((D2, S + 256), u32),
            pltpu.VMEM((S, TQ), f32),
            pltpu.VMEM((S, TQ), f32),
            pltpu.VMEM((S, TQ), f32),
            pltpu.VMEM((H * HP, S), f32),
            pltpu.VMEM((D2, XSPLIT[1]), u32),
            pltpu.VMEM((1, S), f32),
            pltpu.VMEM((7, D2 // 2, H * HP // 2), u32),
            pltpu.VMEM((2, 4, D2, T2), f32),
            pltpu.VMEM((7, D2 // 2, D2), u32),
        ],
        compiler_params=pltpu.CompilerParams(vmem_limit_bytes=100 * 1024 * 1024),
    )(A_x.reshape(S, D).T, A_wqkv, A_wo, B_w1, B_w2, B_w3, B_w4.T, gate_w)
    return out_t.T.reshape(A_x.shape)
```

```python
import math

import jax
import jax.numpy as jnp
from jax import lax
import jax.experimental.pallas as pl
import jax.experimental.pallas.tpu as pltpu

S, D, H, DH, F = 2048, 448, 16, 28, 1792
GW = 4 * DH
HP = 32
HW = HP // 2
TT = 512
TQ = 512
CK = 128
LAG = 2
CATCH = 12
FC = 256
U = 9
PU = 2
NB = 3
C4 = D // 4
D2, F2, T2 = D // 2, FC // 2, TT // 2
NT = S // TT
NSTEP = (S // TQ) * H
NC = S // CK
XSPLIT = (0, 256, 1024, 2048)
KSPLIT = ((0, 256), (256, D))

bf16 = jnp.bfloat16
f32 = jnp.float32
u32 = jnp.uint32

_LHS = ((0, 3, 1), (2, 3, 1), (0, None, 0), (3, None, 0), (0, 1, 1), (2, 0, -1), (1, 3, -1))
_RHS = ((0, 3, 1), (0, None, 0), (1, 3, -1), (2, 0, -1), (3, None, 0), (0, 1, 1), (2, 3, 1))


def _gelu(x, half=0.5):
    c0 = math.sqrt(2.0 / math.pi)
    inner = x * (c0 + (c0 * 0.044715) * (x * x))
    hx = half * x
    return hx + hx * jnp.tanh(inner)


def _ln_t(x):
    m = jnp.sum(x, axis=0, keepdims=True) * (1.0 / D)
    xc = x - m
    v = jnp.sum(xc * xc, axis=0, keepdims=True) * (1.0 / D)
    return xc * lax.rsqrt(v + 1e-5)


def _pk(x):
    return pltpu.bitcast(x.astype(bf16), u32)


def _up(x):
    return pltpu.bitcast(x, bf16)


def _dot(a, b):
    return jnp.dot(a, b, preferred_element_type=f32)


def _operand(term, quad):
    a, b, sign = term
    if sign == 0:
        return quad(a).astype(bf16)
    ta, tb = quad(a).astype(f32), quad(b).astype(f32)
    return (ta + tb if sign > 0 else ta - tb).astype(bf16)


def _strassen(prod, st, emit):
    st[0] = prod(4)
    m3 = prod(2)
    emit(1, st[0] + m3)
    st[3] = m3
    st[1] = prod(1)
    m4 = prod(3)
    emit(2, st[1] + m4)
    st[2] = m4 - st[0]
    st[2] += prod(6)
    m1 = prod(0)
    emit(0, st[2] + m1)
    st[3] = st[3] - st[1] + m1
    emit(3, st[3] + prod(5))


def _span(c0, w, align=128):
    return slice(c0, c0 + w) if isinstance(c0, int) else pl.ds(pl.multiple_of(c0, align), w)


def _chunk_order():
    ntot = U * NC
    order = []
    done = 0
    for n in range(ntot):
        if n >= ntot - CATCH:
            k = n - (ntot - CATCH) + 1
            target = min(n - LAG + (k * (LAG + 1) + CATCH - 1) // CATCH, ntot)
            while done < target:
                order.append((1, done))
                done += 1
            order.append((0, n))
        else:
            order.append((0, n))
            while done <= n - LAG:
                order.append((1, done))
                done += 1
    assert done == ntot
    return order


def _kernel(xt_hbm, wqkv_hbm, wo_hbm, w1_hbm, w2_hbm, w3_hbm, w4t_hbm, gw_hbm, out_hbm,
            xt_v, wqkv_v, wo_v, w1_v, w2_v, w3_v, w4t_v, gw_v, out_v, sems, out_sem, bar_sem,
            w1t_s, wvt_s, wqkt_s, w2t_s, w3k_s, w4k_s, wot_s, gw_s,
            g_s, macc_s, st_s, lnf_s, b_s,
            xp_s, qt_s, k_s, vt_s, h_s, s0_s, s1_s, s2_s, ot_s, ln0_s, gate_s, wok_s, sto_s, wvk_s):
    def cp(src, dst, n):
        return pltpu.make_async_copy(src, dst, sems.at[n])

    def cpx(i, n):
        return cp(xt_hbm.at[:, XSPLIT[i]:XSPLIT[i + 1]], xt_v.at[:, XSPLIT[i]:XSPLIT[i + 1]], n)

    cp_x0 = cpx(0, 0)
    cp_w1 = cp(w1_hbm, w1_v, 1)
    cp_wv = cp(wqkv_hbm.at[:, 2 * D:3 * D], wqkv_v.at[:, 2 * D:3 * D], 2)
    cp_gw = cp(gw_hbm, gw_v, 2)
    cp_x1 = cpx(1, 0)
    cp_x2 = cpx(2, 1)
    cp_wqk = cp(wqkv_hbm.at[:, 0:2 * D], wqkv_v.at[:, 0:2 * D], 1)
    cp_w2 = cp(w2_hbm, w2_v, 1)
    cp_w3a = cp(w3_hbm.at[:, 0:FC], w3_v.at[:, 0:FC], 1)
    cp_wo = cp(wo_hbm, wo_v, 2)
    cp_w3 = cp(w3_hbm.at[:, FC:F], w3_v.at[:, FC:F], 0)
    cp_w4 = cp(w4t_hbm, w4t_v, 0)

    def fence():
        pl.semaphore_signal(bar_sem, 1)
        pl.semaphore_wait(bar_sem, 1)

    cp_x0.start()
    fence()
    cp_w1.start()
    fence()
    cp_wv.start()
    cp_gw.start()

    qscale = (DH ** -0.5) * math.log2(math.e)

    def ln1(c0, w):
        return _ln_t(xt_v[:, c0:c0 + w].astype(f32))

    def put_h(c0, y):
        h_s[:, c0 + 128:c0 + 128 + y.shape[1]] = _pk(_gelu(y))

    def put_v(c0, y, h0=0):
        w = y.shape[1]
        rid = lax.broadcasted_iota(jnp.int32, (HP - DH, w), 0)
        tail = jnp.where(rid == 0, 1.0, 0.0).astype(f32)
        for h in range(y.shape[0] // DH):
            vt_s[HW * (h0 + h):HW * (h0 + h + 1), c0:c0 + w] = _pk(
                jnp.concatenate([y[DH * h:DH * (h + 1), :], tail], axis=0))

    def first_use(w_ref, c0, wt_ref, rhs):
        y = None
        for k0, k1 in KSPLIT:
            wt = w_ref[k0:k1, c0:c0 + D].T
            wt_ref[:, k0:k1] = _pk(wt)
            part = _dot(wt, rhs[k0:k1, :])
            y = part if y is None else y + part
        return y

    def prep_up(c):
        for k in range(7):
            w3k_s[k] = _pk(_operand(_LHS[k], lambda q: w3_v[(q % 2) * D2:(q % 2 + 1) * D2,
                                                            _span(c * FC + (q // 2) * F2, F2)]).T)

    def prep_down(c):
        for k in range(7):
            w4k_s[k] = _pk(_operand(_LHS[k], lambda q: w4t_v[(q // 2) * D2:(q // 2 + 1) * D2,
                                                             _span(c * FC + (q % 2) * F2, F2)]))

    def stage_v(c0, w, slot=0):
        xp_s[:, c0:c0 + w] = _pk(xt_v[:, c0:c0 + w])
        if w < TT:
            put_v(c0, _dot(_up(wvt_s[0]), xt_v[0:D2, c0:c0 + w]) + _dot(_up(wvt_s[1]), xt_v[D2:D, c0:c0 + w]))
            return

        def prod(k):
            return _dot(_up(wvk_s[k]), _operand(
                _RHS[k], lambda q: xt_v[(q // 2) * D2:(q // 2 + 1) * D2,
                                        c0 + (q % 2) * T2:c0 + (q % 2 + 1) * T2]))

        _strassen(prod, sto_s.at[slot], lambda q, c: put_v(c0 + (q % 2) * T2, c, (q // 2) * (H // 2)))

    def stage_h(c0, w):
        xf = xt_v[:, c0:c0 + w].astype(f32)
        gate_s[:, c0:c0 + w] = gate_of(xf)
        put_h(c0, _dot(_up(w1t_s[...]), _ln_t(xf).astype(bf16)))

    def gate_of(x):
        gwc = gw_s[...]
        z = jnp.sum(x.astype(f32) * jnp.concatenate([gwc] * (x.shape[1] // 128), axis=1), axis=0, keepdims=True)
        return 1.0 / (1.0 + jnp.exp(-z))

    h_s[:, 0:128] = jnp.zeros((D2, 128), u32)
    h_s[:, S + 128:S + 256] = jnp.zeros((D2, 128), u32)
    for sb in (s1_s, s2_s):
        sb[0:8, :] = jnp.zeros((8, TQ), f32)
    g_s[0, 0:8, 0:128] = jnp.zeros((8, 128), f32)
    w4k_s[0, 0:8, 0:128] = jnp.zeros((8, 128), u32)
    st_s[0, 0, 0:8, 0:128] = jnp.zeros((8, 128), f32)
    sto_s[0, 0, 0:8, 0:128] = jnp.zeros((8, 128), f32)
    wok_s[0, 0:8, 0:128] = jnp.zeros((8, 128), u32)
    for k in (0, 1, 2, 3):
        macc_s[k] = jnp.zeros(macc_s.shape[1:], f32)
    w0 = XSPLIT[1]
    cp_x0.wait()
    cp_x1.start()
    macc_s[4] = jnp.zeros(macc_s.shape[1:], f32)
    ln0_s[...] = _pk(ln1(0, w0))
    cp_w1.wait()
    put_h(0, first_use(w1_v, 0, w1t_s, _up(ln0_s[...])))
    cp_wv.wait()
    cp_gw.wait()
    cp_x2.start()
    wv_t = [wqkv_v[j * D2:(j + 1) * D2, 2 * D:3 * D].T for j in range(2)]
    for j in range(2):
        wvt_s[j] = _pk(wv_t[j])
    put_v(0, _dot(wv_t[0], xt_v[0:D2, 0:w0]) + _dot(wv_t[1], xt_v[D2:D, 0:w0]))
    xp_s[:, 0:w0] = _pk(xt_v[:, 0:w0])
    gw_s[...] = jnp.broadcast_to(gw_v[...].astype(f32).reshape(1, D), (128, D)).T
    cp_x1.wait()
    cp_wqk.start()
    cp_w2.start()
    cp_w3a.start()
    for k in (4, 2, 1, 3, 6, 0, 5):
        wvk_s[k] = _pk(_operand(
            _LHS[k], lambda q: _up(wvt_s[q % 2, (q // 2) * D2 // 2:(q // 2 + 1) * D2 // 2, :])))
    stage_v(256, 256)
    stage_h(256, 256)
    stage_h(512, 512)
    stage_v(512, 512)
    gate_s[:, 0:w0] = gate_of(xt_v[:, 0:w0])
    cp_x2.wait()
    cp_wqk.wait()
    cp_w2.wait()
    cp_w3a.wait()
    cp_wo.start()
    fence()
    cp_w3.start()
    cp_w4.start()
    prep_up(0)
    wqkt_s[...] = _pk(wqkv_v[:, 0:2 * D].T)
    w2t_s[...] = _pk(w2_v[...].T)
    stage_v(1024, 512)
    stage_h(1024, 512)
    stage_h(1536, 512)
    stage_v(1536, 512, 1)
    cp_wo.wait()

    def proj(i, odd, m):
        cols = _span(i * TT, TT)
        xt = _up(xp_s[:, cols])
        zpad = jnp.zeros((HP - DH, TT), f32)

        def heads(y, n):
            return [jnp.concatenate([y[DH * h:DH * (h + 1), :], zpad], axis=0).astype(bf16) for h in range(n)]

        kn = [kh.T for kh in heads(_dot(_up(wqkt_s[D2:D, :]), xt), H)]
        for h in range(H):
            k_s[h, _span(i * T2, T2), :] = _pk(kn[h])
        hw = h_s[:, _span(i * TT, TT + 256)]
        c8 = C4 // 2
        hs = _up(jnp.concatenate([
            hw[0 * c8:1 * c8, 127:127 + TT],
            hw[1 * c8:2 * c8, 129:129 + TT],
            hw[2 * c8:3 * c8, 126:126 + TT],
            hw[3 * c8:4 * c8, 130:130 + TT]], axis=0))

        def qproj(h0, h1):
            y = _dot(_up(wqkt_s[h0 * DH // 2:h1 * DH // 2, :]), xt) * qscale
            for h, qh in enumerate(heads(y, h1 - h0)):
                qt_s[HW * (h + h0):HW * (h + h0 + 1), cols] = _pk(qh)

        qproj(0, 4)
        x1 = xt.astype(f32) + _dot(_up(w2t_s[...]), hs)
        hcols = _span((i - odd) * T2, TT)
        xs = x1 * (1.0 - gate_s[:, cols])
        if odd:
            b_s[0, :, hcols] = xs[0:D2, :]
            macc_s[5, :, hcols] = xs[D2:D, :]
        else:
            macc_s[6, :, hcols] = xs[0:D2, :]
            b_s[1, :, hcols] = xs[D2:D, :]
        lnf_s[:, cols] = _ln_t(x1)
        s = _dot(kn[0], _up(qt_s[0:HW, 0:TQ]))
        s0_s[cols, :] = s
        m = jnp.maximum(m, jnp.max(s.reshape(TT // 8, 8, TQ), axis=0))
        qproj(4, H)
        wo_f = wo_v[_span(i * GW, GW, 16), :].astype(f32)
        zrows = jnp.zeros((HP - DH, D), f32)
        parts = []
        for j in range(4):
            parts += [wo_f[DH * j:DH * (j + 1), :], zrows]
        wot_s[:, _span(i * 128, 128)] = _pk(jnp.concatenate(parts, axis=0).astype(bf16).T)
        return m

    def proj_body(ii, m):
        for u in range(PU):
            m = proj(ii * PU + u, u % 2, m)
        return m

    m = lax.fori_loop(0, NT // PU, proj_body, jnp.full((8, TQ), -jnp.inf, f32))
    cp_w3.wait()
    cp_w4.wait()

    sbuf = (s0_s, s1_s, s2_s)

    def ffn_up(p):
        def prod(k):
            return _dot(_up(w3k_s[k]), _operand(
                _RHS[k], lambda q: lnf_s[(q // 2) * D2:(q // 2 + 1) * D2,
                                         (2 * p + q % 2) * TT:(2 * p + q % 2 + 1) * TT]))

        def emit(q, c):
            tb = 2 * p + q % 2
            g_s[q, :, p * TT:(p + 1) * TT] = _gelu(c, 0.5 - 0.5 * gate_s[:, tb * TT:(tb + 1) * TT])

        _strassen(prod, st_s.at[p], emit)

    def ffn_down(p):
        cols = slice(p * TT, (p + 1) * TT)
        for k in (1, 3, 5, 0, 2, 4, 6):
            macc_s[k, :, cols] += _dot(_up(w4k_s[k]), _operand(_RHS[k], lambda q: g_s[q, :, cols]))

    def body(i, m_in):
        extra = {0: lambda: prep_down(i), 1: lambda: ffn_up(0), 2: lambda: ffn_up(1),
                 3: lambda: ffn_down(0), 4: lambda: ffn_down(1),
                 5: lambda: prep_up(jnp.minimum(i + 1, F // FC - 1))}
        mx = {-1: m_in}
        mrow = {}
        qms = {}
        accs = {}
        for kind, n in _chunk_order():
            u, cc = divmod(n, NC)
            if kind == 0 and cc == LAG and u in extra:
                extra[u]()
            ks = slice(cc * CK, (cc + 1) * CK)
            if kind == 0:
                t1 = i * U + u + 1
                h1 = t1 & (H - 1)
                if cc == 0:
                    qms[u] = _up(qt_s[_span(h1 * HW, HW, HW), _span((t1 >> 4) * TQ, TQ)])
                s = _dot(_up(k_s[h1, cc * CK // 2:(cc + 1) * CK // 2, :]), qms[u])
                sbuf[(u + 1) % NB][ks, :] = s
                mc = jnp.max(s.reshape(CK // 8, 8, TQ), axis=0)
                mx[u] = mc if cc == 0 else jnp.maximum(mx[u], mc)
            else:
                t2 = i * U + u
                hrows = _span((t2 & (H - 1)) * HW, HW, HW)
                if cc == 0:
                    mrow[u] = jnp.max(mx[u - 1], axis=0, keepdims=True)
                p = jnp.exp2(sbuf[u % NB][ks, :] - mrow[u]).astype(bf16)
                pv = _dot(_up(vt_s[hrows, ks]), p)
                accs[u] = pv if cc == 0 else accs[u] + pv
                if cc == NC - 1:
                    acc = accs[u]
                    qcols = _span((t2 >> 4) * TQ, TQ)
                    inv = gate_s[:, qcols] / acc[DH:DH + 1, :]
                    ot_s[hrows, qcols] = _pk(acc * inv)
        return mx[U - 1]

    m = lax.fori_loop(0, (NSTEP - 1) // U, body, m)

    s_last = sbuf[(NSTEP - 1) % NB]
    m_last = jnp.max(m, axis=0, keepdims=True)

    def last_pv():
        pacc = None
        for cc in range(NC):
            ks = slice(cc * CK, (cc + 1) * CK)
            p = jnp.exp2(s_last[ks, :] - m_last).astype(bf16)
            pv = _dot(_up(vt_s[(H - 1) * HW:H * HW, ks]), p)
            pacc = pv if pacc is None else pacc + pv
            if cc == NC - 1:
                inv = gate_s[:, S - TQ:S] / pacc[DH:DH + 1, :]
                ot_s[(H - 1) * HW:H * HW, S - TQ:S] = _pk(pacc * inv)
            yield

    pvs = last_pv()
    KH = H * HP // 2
    for k in (4, 2, 1, 3, 6, 0, 5):
        wok_s[k] = _pk(_operand(
            _LHS[k], lambda q: _up(wot_s[(q // 2) * D2 // 2:(q // 2 + 1) * D2 // 2,
                                         (q % 2) * KH:(q % 2 + 1) * KH])))
    nprod = [0]

    def out_pair(p, j):
        hc = slice(p * TT + j * T2, p * TT + (j + 1) * T2)

        def tcols(q):
            c0 = (2 * p + q % 2) * TT + j * T2
            return slice(c0, c0 + T2)

        def prod(k):
            rhs = _operand(_RHS[k], lambda q: _up(ot_s[(q // 2) * KH // 2:(q // 2 + 1) * KH // 2, tcols(q)]))
            cuts = (0, 40, 80, D2 // 2) if nprod[0] < NC // 2 else (0, D2 // 2)
            nprod[0] += 1
            parts = []
            for a, b in zip(cuts[:-1], cuts[1:]):
                if a:
                    next(pvs)
                parts.append(_dot(_up(wok_s[k, a:b, :]), rhs))
            return macc_s[k, :, hc] + jnp.concatenate(parts, axis=0)

        def emit(q, c):
            rows = slice((q // 2) * D2, (q // 2 + 1) * D2)
            if q in (1, 2):
                c = c + b_s[q - 1, :, hc]
            out_v[rows, tcols(q)] = c.astype(bf16)
            pltpu.make_async_copy(out_v.at[rows, tcols(q)], out_hbm.at[rows, tcols(q)], out_sem).start()

        _strassen(prod, sto_s.at[j], emit)

    for p in range(2):
        for j in range(2):
            out_pair(p, j)
    pltpu.make_async_copy(out_v, out_hbm, out_sem).wait()


@jax.jit
def pallas_gated_mix__mha_block__mixer_s_mlp__prompt_kernel(
    A_x: jax.Array,
    A_wqkv: jax.Array,
    A_wo: jax.Array,
    B_x: jax.Array,
    B_w1: jax.Array,
    B_w2: jax.Array,
    B_w3: jax.Array,
    B_w4: jax.Array,
    gate_w: jax.Array,
):
    del B_x
    any_spec = pl.BlockSpec(memory_space=pl.ANY)
    out_t = pl.pallas_call(
        _kernel,
        out_shape=jax.ShapeDtypeStruct((D, S), A_x.dtype),
        in_specs=[any_spec] * 8,
        out_specs=any_spec,
        scratch_shapes=[
            pltpu.VMEM((D, S), bf16),
            pltpu.VMEM((D, 3 * D), bf16),
            pltpu.VMEM((D, D), bf16),
            pltpu.VMEM((D, D), bf16),
            pltpu.VMEM((D, D), bf16),
            pltpu.VMEM((D, F), bf16),
            pltpu.VMEM((D, F), bf16),
            pltpu.VMEM((D,), bf16),
            pltpu.VMEM((D, S), bf16),
            pltpu.SemaphoreType.DMA((3,)),
            pltpu.SemaphoreType.DMA(()),
            pltpu.SemaphoreType.REGULAR,
            pltpu.VMEM((D2, D), u32),
            pltpu.VMEM((2, D2, D2), u32),
            pltpu.VMEM((D, D), u32),
            pltpu.VMEM((D2, D), u32),
            pltpu.VMEM((7, F2 // 2, D2), u32),
            pltpu.VMEM((7, D2 // 2, F2), u32),
            pltpu.VMEM((D2, H * HP), u32),
            pltpu.VMEM((D, 128), f32),
            pltpu.VMEM((4, F2, S // 2), f32),
            pltpu.VMEM((7, D2, S // 2), f32),
            pltpu.VMEM((2, 4, F2, TT), f32),
            pltpu.VMEM((D, S), f32),
            pltpu.VMEM((2, D2, S // 2), f32),
            pltpu.VMEM((D2, S), u32),
            pltpu.VMEM((H * HW, S), u32),
            pltpu.VMEM((H, S // 2, HP), u32),
            pltpu.VMEM((H * HW, S), u32),
            pltpu.VMEM((D2, S + 256), u32),
            pltpu.VMEM((S, TQ), f32),
            pltpu.VMEM((S, TQ), f32),
            pltpu.VMEM((S, TQ), f32),
            pltpu.VMEM((H * HW, S), u32),
            pltpu.VMEM((D2, XSPLIT[1]), u32),
            pltpu.VMEM((1, S), f32),
            pltpu.VMEM((7, D2 // 2, H * HP // 2), u32),
            pltpu.VMEM((2, 4, D2, T2), f32),
            pltpu.VMEM((7, D2 // 2, D2), u32),
        ],
        compiler_params=pltpu.CompilerParams(vmem_limit_bytes=100 * 1024 * 1024),
    )(A_x.reshape(S, D).T, A_wqkv, A_wo, B_w1, B_w2, B_w3, B_w4.T, gate_w)
    return out_t.T.reshape(A_x.shape)
```
